```python
import os as _os
_os.environ.setdefault("JAX_PLATFORMS", "cpu")
import jax
import jax.numpy as jnp

def _softmax(x, axis=-1):
    return jax.nn.softmax(x, axis=axis)
def _gelu(x):
    return jax.nn.gelu(x, approximate=True)
def _silu(x):
    return jax.nn.silu(x)
def _sigmoid(x):
    return jax.nn.sigmoid(x)
def _layernorm(x, axis=-1, eps=1e-5):
    m = jnp.mean(x, axis=axis, keepdims=True)
    v = jnp.var(x, axis=axis, keepdims=True)
    return (x - m) / jnp.sqrt(v + eps)
def _scatter_add(tgt, idx, src, axis=0):
    return tgt.at[idx].add(src)
def _segment_sum(src, seg, n):
    return jax.ops.segment_sum(src, seg, n)
class _Rng:
    def __init__(self, key):
        self._k = key
    def _next(self):
        self._k, sub = jax.random.split(self._k)
        return sub
    def normal(self, shape):
        return jax.random.normal(self._next(), shape, dtype=jnp.bfloat16)
    def randint(self, lo, hi, shape):
        return jax.random.randint(self._next(), shape, lo, hi, dtype=jnp.int32)
    def uniform(self, shape, lo=0.0, hi=1.0):
        return jax.random.uniform(self._next(), shape, jnp.bfloat16, lo, hi)
    def permutation(self, n):
        return jax.random.permutation(self._next(), n)


kernel_name = 'parallel_sum__ssm_conv_s5__glu_gated_swiglu__prompt'

def setup_inputs():
    _rng = _Rng(jax.random.key(int.from_bytes(__import__("os").urandom(4), "little")))
    _w = (lambda a: (lambda t: t.astype(jnp.bfloat16) if jnp.issubdtype(t.dtype, jnp.floating) else t)(jnp.asarray(a)))
    def _A_setup():
        B, S, D = 1, 2048, 640
        P = D
        Lambda_re = -0.5 * jnp.exp((lambda *s: _rng.normal(s) * 0.4)(P))
        Lambda_im = (lambda *s: _rng.normal(s) * 0.4)(P) * 1.0
        B_re = (lambda *s: _rng.normal(s) * 0.4)(P, D) * (D ** -0.5)
        B_im = (lambda *s: _rng.normal(s) * 0.4)(P, D) * (D ** -0.5)
        C_re = (lambda *s: _rng.normal(s) * 0.4)(D, P) * (P ** -0.5)
        C_im = (lambda *s: _rng.normal(s) * 0.4)(D, P) * (P ** -0.5)
        log_dt = (lambda *s: _rng.normal(s) * 0.4)(P) * 0.3 - 2.0
        Dskip = (lambda *s: _rng.normal(s) * 0.4)(D)
        return {
            "x": _w((lambda *s: _rng.normal(s) * 0.05)(B, S, D)),
            "Lambda_re": _w(Lambda_re),
            "Lambda_im": _w(Lambda_im),
            "B_re": _w(B_re),
            "B_im": _w(B_im),
            "C_re": _w(C_re),
            "C_im": _w(C_im),
            "log_dt": _w(log_dt),
            "Dskip": _w(Dskip),
        }
    _A_in = _A_setup()

    def _B_setup():
        B, S, D, F = 1, 2048, 640, 1728
        return {
            "x": _w((lambda *s: _rng.normal(s) * 0.05)(B, S, D)),
            "w1": _w((lambda *s: _rng.normal(s) * 0.1)(D, F) * (2.0 / D) ** 0.5),
            "w3": _w((lambda *s: _rng.normal(s) * 0.1)(D, F) * (2.0 / D) ** 0.5),
            "w2": _w((lambda *s: _rng.normal(s) * 0.1)(F, D) * (2.0 / F) ** 0.5),
        }
    _B_in = _B_setup()

    return {
        "A_x": _A_in["x"],
        "A_Lambda_re": _A_in["Lambda_re"],
        "A_Lambda_im": _A_in["Lambda_im"],
        "A_B_re": _A_in["B_re"],
        "A_B_im": _A_in["B_im"],
        "A_C_re": _A_in["C_re"],
        "A_C_im": _A_in["C_im"],
        "A_log_dt": _A_in["log_dt"],
        "A_Dskip": _A_in["Dskip"],
        "B_x": _B_in["x"],
        "B_w1": _B_in["w1"],
        "B_w3": _B_in["w3"],
        "B_w2": _B_in["w2"],
    }

def reference(A_x, A_Lambda_re, A_Lambda_im, A_B_re, A_B_im, A_C_re, A_C_im, A_log_dt, A_Dskip, B_x, B_w1, B_w3, B_w2):
    def _A_ref(x, Lambda_re, Lambda_im, B_re, B_im, C_re, C_im, log_dt, Dskip):
        Bsz, L, H = x.shape
        Lam = Lambda_re + 1j * Lambda_im
        Bmat = B_re + 1j * B_im
        Cmat = C_re + 1j * C_im
        dt = jnp.exp(log_dt)
        Lam_bar = jnp.exp(dt * Lam)
        B_bar = ((Lam_bar - 1.0) / Lam)[:, None] * Bmat
        Bu = jnp.einsum("bld,pd->blp", x + 0j, B_bar)
        h = jnp.zeros_like(Bu[:, 0, :])
        hs = []
        for t in range(L):
            h = Lam_bar[None, :] * h + Bu[:, t, :]
            hs.append(h)
        hseq = jnp.stack(hs, 1)
        y = 2.0 * jnp.einsum("blp,dp->bld", hseq, Cmat).real + x * Dskip[None, None, :]
        return y

    def _B_ref(x, w1, w3, w2):
        gate = jnp.einsum("bsd,df->bsf", x, w1)
        up = jnp.einsum("bsd,df->bsf", x, w3)
        h = _silu(gate) * up
        out = jnp.einsum("bsf,fd->bsd", h, w2)
        return out

    x = A_x
    xn = _layernorm(x, axis=-1)
    return x + _A_ref(xn, A_Lambda_re, A_Lambda_im, A_B_re, A_B_im, A_C_re, A_C_im, A_log_dt, A_Dskip) + _B_ref(xn, B_w1, B_w3, B_w2)
```

```python
import jax
import jax.numpy as jnp
from jax import lax
import jax.experimental.pallas as pl
import jax.experimental.pallas.tpu as pltpu

F32 = jnp.float32
BF16 = jnp.bfloat16
I32 = jnp.int32
NT = (((1,), (1,)), ((), ()))


def _cmul(ar, ai, br, bi):
    return ar * br - ai * bi, ar * bi + ai * br


def _swiglu(g, u):
    hg = 0.5 * g
    return ((hg * jnp.tanh(hg) + hg) * u).astype(BF16)


def _or_all(vs):
    acc = vs[0]
    for v in vs[1:]:
        acc = acc | v
    return acc


def _pin(lhs, link):
    if link is None:
        return lhs
    blk = pltpu.bitcast(pltpu.bitcast(lhs[0:16, 0:128], I32) | link, BF16)
    top = jnp.concatenate([blk, lhs[0:16, 128:]], axis=1) if lhs.shape[1] > 128 else blk
    return jnp.concatenate([top, lhs[16:, :]], axis=0)


def _pin32(v, link):
    if link is None:
        return v
    blk = pltpu.bitcast(pltpu.bitcast(v[0:8, :], I32) | link, F32)
    return jnp.concatenate([blk, v[8:, :]], axis=0)


def make(T=256, NA=7, ND=3, RB=32, ORD='S-S-S-S-S----', LP=(1, 1, 1, 1, 1, 1, 1, 1, 0, 0), MID=False):
    S = T // 8
    PITCH = S + 4
    NB = T // RB

    def kernel(x_hbm, lre_hbm, lim_hbm, ldt_hbm, dsk_hbm, bre_hbm, bim_hbm, cre_hbm, cim_hbm,
               w1_hbm, w3_hbm, w2_hbm, o_ref,
               x_v, par_v, b_v, c_v, w1_v, w3_v, wt_v, w2_v,
               xin_scr, xout_scr, xn_scr, base_scr, xn0_scr, base0_scr, raw0_scr, dsk_scr,
               lam_scr, pw_scr, cp_scr, carry_scr, raw_scr, zero_scr,
               w_sem):
        L, D = x_v.shape
        P = b_v.shape[1]
        Fh = w2_v.shape[0]
        Fm = (Fh // 128) * 128
        Ft = Fh - Fm
        NG = Fm // 128
        NL = D // 128
        NP = P // 128
        NC = L // T
        i = pl.program_id(0)

        NW = 15

        def x_copy(c):
            return pltpu.make_async_copy(x_hbm.at[0, pl.ds(c * T, T), :], x_v.at[pl.ds(c * T, T), :], w_sem.at[NW + c])

        cps = {}
        def add(name, src, dst):
            cps[name] = pltpu.make_async_copy(src, dst, w_sem.at[len(cps)])
        for k, r in enumerate((dsk_hbm, lre_hbm, lim_hbm, ldt_hbm)):
            add(('par', k), r, par_v.at[k])
        add('bre', bre_hbm, b_v.at[0])
        add('bim', bim_hbm, b_v.at[1])
        FA = NA * 128
        add('w1a', w1_hbm.at[pl.ds(0, FA), :], w1_v.at[pl.ds(0, FA), :])
        add('w3a', w3_hbm.at[pl.ds(0, FA), :], w3_v.at[pl.ds(0, FA), :])
        add('w1b', w1_hbm.at[pl.ds(FA, Fm - FA), :], w1_v.at[pl.ds(FA, Fm - FA), :])
        add('w3b', w3_hbm.at[pl.ds(FA, Fm - FA), :], w3_v.at[pl.ds(FA, Fm - FA), :])
        add('wt1', w1_hbm.at[pl.ds(Fm, Ft), :], wt_v.at[pl.ds(0, Ft), :])
        add('wt3', w3_hbm.at[pl.ds(Fm, Ft), :], wt_v.at[pl.ds(Ft, Ft), :])
        add('w2', w2_hbm, w2_v)
        add('cre', cre_hbm, c_v.at[0])
        add('cim', cim_hbm, c_v.at[1])
        wait = lambda *names: [cps[n].wait() for n in names]

        def ln_stage(c):
            start = c * T if isinstance(c, int) else pl.multiple_of(c * T, T)
            xf = x_v[pl.ds(start, T), :].astype(F32)
            for j in range(NL):
                for s in range(8):
                    xin_scr[j, pl.ds(PITCH * s, S), :] = xf[S * s:S * (s + 1), 128 * j:128 * (j + 1)]

        def ln_block(r):
            ts = range(r * RB // 8, (r + 1) * RB // 8)
            xp = jnp.concatenate(
                [jnp.concatenate([xin_scr[j, pl.ds(t, 8, stride=PITCH), :] for t in ts], axis=0)
                 for j in range(NL)], axis=1)
            mean = jnp.sum(xp, axis=-1, keepdims=True) * (1.0 / D)
            xc = xp - mean
            var = jnp.sum(xc * xc, axis=-1, keepdims=True) * (1.0 / D)
            m_b = mean.astype(BF16).astype(F32)
            v_b = var.astype(BF16).astype(F32)
            sd = jnp.sqrt((v_b + 1e-5).astype(BF16).astype(F32)).astype(BF16).astype(F32)
            xn = ((xp - m_b) * (1.0 / sd)).astype(BF16)
            base = xp + xn.astype(F32) * dsk_scr[0:1, :]
            bi = pltpu.bitcast(base, I32)
            link = _or_all([bi[8 * a:8 * a + 8, 128 * j:128 * (j + 1)] for a in range(RB // 8) for j in range(NL)])
            return xn, base, link & zero_scr[...]

        def ln_full(c, xn_dst, base_dst):
            ln_stage(c)
            for r in range(NB):
                xn, base, _ = ln_block(r)
                xn_dst[r * RB:(r + 1) * RB, :] = xn
                base_dst[r * RB:(r + 1) * RB, :] = base

        def row_table(v):
            return jnp.concatenate([jnp.broadcast_to(v[j:j + 1, :], (8, 128)) for j in range(v.shape[0])], axis=1)

        def prep_params():
            dsk_scr[...] = row_table(par_v[0].astype(F32))
            lr = par_v[1].astype(F32)
            li = par_v[2].astype(F32)
            dt = jnp.exp(par_v[3].astype(F32)).astype(BF16).astype(F32)
            a = dt * lr
            b = dt * li
            mag = jnp.exp(a)
            lbr = mag * jnp.cos(b)
            lbi = mag * jnp.sin(b)
            nr = lbr - 1.0
            ni = lbi
            big = jnp.abs(lr) >= jnp.abs(li)
            r1 = li / lr
            d1 = lr + li * r1
            r2 = lr / li
            d2 = lr * r2 + li
            cr = jnp.where(big, (nr + ni * r1) / d1, (nr * r2 + ni) / d2)
            ci = jnp.where(big, (ni - nr * r1) / d1, (ni * r2 - nr) / d2)
            lam_scr[0] = row_table(lbr)
            lam_scr[1] = row_table(lbi)
            lam_scr[2] = row_table(2.0 * cr)
            lam_scr[3] = row_table(2.0 * ci)
            pr, pi = lbr, lbi
            n = 1
            while n < S:
                pr, pi = _cmul(pr, pi, pr, pi)
                n *= 2
            for k in range(3):
                pw_scr[2 * k] = row_table(pr)
                pw_scr[2 * k + 1] = row_table(pi)
                pr, pi = _cmul(pr, pi, pr, pi)
            carry_scr[...] = jnp.zeros(carry_scr.shape, F32)
            zero_scr[...] = jnp.zeros(zero_scr.shape, I32)

        def prep_c():
            cr = lam_scr[2, 0:1, :]
            ci = lam_scr[3, 0:1, :]
            RC = 64
            for r in range(0, D, RC):
                c_r = c_v[0, r:r + RC, :].astype(F32)
                c_i = c_v[1, r:r + RC, :].astype(F32)
                cp_scr[r:r + RC, :P] = (c_r * cr - c_i * ci).astype(BF16)
                cp_scr[r:r + RC, P:] = (-(c_r * ci) - c_i * cr).astype(BF16)

        def scan_tile(j, raw):
            sub = lax.broadcasted_iota(I32, (8, 128), 0)
            cr_ = slice(128 * j, 128 * (j + 1))
            ci_ = slice(P + 128 * j, P + 128 * (j + 1))
            lbr = lam_scr[0, :, cr_]
            lbi = lam_scr[1, :, cr_]
            er = raw[0:8, cr_]
            ei = raw[0:8, ci_]
            for t in range(1, S):
                ur = raw[8 * t:8 * t + 8, cr_]
                ui = raw[8 * t:8 * t + 8, ci_]
                er, ei = (lbr * er - lbi * ei) + ur, (lbr * ei + lbi * er) + ui
            vr = pltpu.roll(jnp.where(sub == 7, carry_scr[0, :, cr_], er), 1, 0)
            vi = pltpu.roll(jnp.where(sub == 7, carry_scr[1, :, cr_], ei), 1, 0)
            for k in range(3):
                sh = 1 << k
                ar = pw_scr[2 * k, :, cr_]
                ai = pw_scr[2 * k + 1, :, cr_]
                sr = pltpu.roll(vr, sh, 0)
                si = pltpu.roll(vi, sh, 0)
                tr, ti = _cmul(ar, ai, sr, si)
                msk = sub >= sh
                vr = vr + jnp.where(msk, tr, 0.0)
                vi = vi + jnp.where(msk, ti, 0.0)
            hr, hi = vr, vi
            prs, pis = [], []
            for t2 in range(S // 2):
                outs = []
                for t in (2 * t2, 2 * t2 + 1):
                    ur = raw[8 * t:8 * t + 8, cr_]
                    ui = raw[8 * t:8 * t + 8, ci_]
                    hr, hi = (lbr * hr - lbi * hi) + ur, (lbr * hi + lbi * hr) + ui
                    outs.append((hr, hi))
                prs.append(jnp.concatenate([outs[0][0], outs[1][0]], axis=0).astype(BF16))
                pis.append(jnp.concatenate([outs[0][1], outs[1][1]], axis=0).astype(BF16))
            carry_scr[0, :, cr_] = hr
            carry_scr[1, :, cr_] = hi
            link = _or_all([pltpu.bitcast(v, I32) for pr_pi in zip(prs, pis) for v in pr_pi])
            return jnp.concatenate(prs, axis=0), jnp.concatenate(pis, axis=0), link & zero_scr[...]

        def up_stage(xn_ref, raw, first):
            xn = xn_ref[...]
            hs, g_re, g_im = [], [], []
            for gi in range(NG):
                if first and gi == 0:
                    wait('w1a', 'w3a')
                if first and gi == NA:
                    wait('w1b', 'w3b', 'wt1', 'wt3')
                    xn = xn_ref[...]
                lk = None
                if ORD[gi] == 'S' and len(g_re) < NP:
                    gr, gim, lk = scan_tile(len(g_re), raw)
                    g_re.append(gr)
                    g_im.append(gim)
                rs = slice(128 * gi, 128 * (gi + 1))
                gate = lax.dot_general(xn, w1_v[rs, :], NT, preferred_element_type=F32)
                up = lax.dot_general(xn, w3_v[rs, :], NT, preferred_element_type=F32)
                hs.append(_pin(_swiglu(gate, up), lk))
            tail = lax.dot_general(xn, wt_v[...], NT, preferred_element_type=F32)
            ht = _swiglu(tail[:, :Ft], tail[:, Ft:])
            assert len(g_re) == NP
            return jnp.concatenate(hs, axis=1), ht, jnp.concatenate(g_re + g_im, axis=1)

        def write_out(out):
            for j in range(NL):
                for t in range(S):
                    xout_scr[j, pl.ds(t, 8, stride=PITCH), :] = out[8 * t:8 * t + 8, 128 * j:128 * (j + 1)]
            for j in range(NL):
                for s in range(8):
                    o_ref[S * s:S * (s + 1), 128 * j:128 * (j + 1)] = xout_scr[j, pl.ds(PITCH * s, S), :]

        def main(last):
            if not last:
                ln_stage(i + 1)
            h, ht, g = up_stage(xn_scr, raw_scr, False)
            xns, bases = [], []

            def ln_pin(k):
                lk = None
                if not last:
                    for _ in range(LP[k]):
                        if len(xns) < NB:
                            r = len(xns)
                            xb, bb, l2 = ln_block(r)
                            xn_scr[r * RB:(r + 1) * RB, :] = xb
                            xns.append(xb)
                            bases.append(bb)
                            lk = l2 if lk is None else lk | l2
                return lk

            ys = []
            for n in range(NL):
                cs = slice(128 * n, 128 * (n + 1))
                yn = jnp.dot(h, w2_v[:Fm, cs], preferred_element_type=F32)
                yn = _pin32(yn, ln_pin(2 * n))
                yn = yn + jnp.dot(ht, w2_v[Fm:, cs], preferred_element_type=F32)
                yn = yn + lax.dot_general(g, cp_scr[cs, :], NT, preferred_element_type=F32)
                yn = _pin32(yn, ln_pin(2 * n + 1))
                ys.append(yn)
            y = jnp.concatenate(ys, axis=1)
            if not last:
                assert len(xns) == NB
                xn_next = jnp.concatenate(xns, axis=0)
                raw_scr[:, :P] = lax.dot_general(xn_next, b_v[0], NT, preferred_element_type=F32)
                raw_scr[:, P:] = lax.dot_general(xn_next, b_v[1], NT, preferred_element_type=F32)
            out = base_scr[...] + y
            if not last:
                base_scr[...] = jnp.concatenate(bases, axis=0)
            write_out(out)

        def first_step():
            for k in range(4):
                cps[('par', k)].start()
            x_copy(0).start()
            x_copy(1).start()
            for n in cps:
                if n[0] != 'par':
                    cps[n].start()
            x_copy(2).start()
            wait(*[('par', k) for k in range(4)])
            prep_params()
            x_copy(0).wait()
            ln_full(0, xn0_scr, base0_scr)
            x_copy(1).wait()
            ln_full(1, xn_scr, base_scr)
            for k, nm in enumerate(('bre', 'bim')):
                wait(nm)
                xx = jnp.concatenate([xn0_scr[...], xn_scr[...]], axis=0)
                rr = lax.dot_general(xx, b_v[k], NT, preferred_element_type=F32)
                raw0_scr[:, k * P:(k + 1) * P] = rr[:T]
                raw_scr[:, k * P:(k + 1) * P] = rr[T:]
            if MID:
                wait(*[n for n in cps if n not in ('bre', 'bim') and n[0] != 'par'])
                return
            h, ht, g = up_stage(xn0_scr, raw0_scr, True)
            wait('w2')
            ys = []
            for n in range(NL):
                if n == ND:
                    wait('cre', 'cim')
                    prep_c()
                cs = slice(128 * n, 128 * (n + 1))
                yn = jnp.dot(h, w2_v[:Fm, cs], preferred_element_type=F32)
                yn = yn + jnp.dot(ht, w2_v[Fm:, cs], preferred_element_type=F32)
                ys.append(yn)
            y = jnp.concatenate(ys, axis=1)
            y = y + lax.dot_general(g, cp_scr[...], NT, preferred_element_type=F32)
            write_out(base0_scr[...] + y)

        @pl.when(i == 0)
        def _():
            first_step()

        @pl.when(jnp.logical_and(i > 0, i < NC - 1))
        def _():
            x_copy(i + 1).wait()

            @pl.when(i + 2 < NC)
            def _():
                x_copy(i + 2).start()
            main(False)

        @pl.when(i == NC - 1)
        def _():
            if not MID:
                main(True)

    @jax.jit
    def f(A_x, A_Lambda_re, A_Lambda_im, A_B_re, A_B_im, A_C_re, A_C_im, A_log_dt, A_Dskip, B_x, B_w1, B_w3, B_w2):
        Bsz, L, D = A_x.shape
        P = A_Lambda_re.shape[0]
        Fh = B_w1.shape[1]
        Ft = Fh % 128
        Fm = Fh - Ft
        NC = L // T
        vec = lambda a: a.reshape(-1, 128)
        args = (A_x, vec(A_Lambda_re), vec(A_Lambda_im), vec(A_log_dt), vec(A_Dskip),
                A_B_re, A_B_im, A_C_re, A_C_im, B_w1.T, B_w3.T, B_w2)
        return pl.pallas_call(
            kernel,
            grid=(NC,),
            in_specs=[pl.BlockSpec(memory_space=pl.ANY)] * len(args),
            out_specs=pl.BlockSpec((None, T, D), lambda i: (0, i, 0)),
            out_shape=jax.ShapeDtypeStruct((Bsz, L, D), F32),
            scratch_shapes=[
                pltpu.VMEM((L, D), BF16),
                pltpu.VMEM((4, P // 128, 128), BF16),
                pltpu.VMEM((2, P, D), BF16),
                pltpu.VMEM((2, D, P), BF16),
                pltpu.VMEM((Fm, D), BF16),
                pltpu.VMEM((Fm, D), BF16),
                pltpu.VMEM((2 * Ft, D), BF16),
                pltpu.VMEM((Fh, D), BF16),
                pltpu.VMEM((D // 128, 8 * PITCH, 128), F32),
                pltpu.VMEM((D // 128, 8 * PITCH, 128), F32),
                pltpu.VMEM((T, D), BF16),
                pltpu.VMEM((T, D), F32),
                pltpu.VMEM((T, D), BF16),
                pltpu.VMEM((T, D), F32),
                pltpu.VMEM((T, 2 * P), F32),
                pltpu.VMEM((8, D), F32),
                pltpu.VMEM((4, 8, P), F32),
                pltpu.VMEM((6, 8, P), F32),
                pltpu.VMEM((D, 2 * P), BF16),
                pltpu.VMEM((2, 8, P), F32),
                pltpu.VMEM((T, 2 * P), F32),
                pltpu.VMEM((8, 128), I32),
                pltpu.SemaphoreType.DMA((15 + NC,)),
            ],
            compiler_params=pltpu.CompilerParams(dimension_semantics=("arbitrary",),
                                                 vmem_limit_bytes=100 * 1024 * 1024),
        )(*args)
    return f


_IMPL = make()


@jax.jit
def pallas_parallel_sum__ssm_conv_s5__glu_gated_swiglu__prompt_kernel(
    A_x: jax.Array,
    A_Lambda_re: jax.Array,
    A_Lambda_im: jax.Array,
    A_B_re: jax.Array,
    A_B_im: jax.Array,
    A_C_re: jax.Array,
    A_C_im: jax.Array,
    A_log_dt: jax.Array,
    A_Dskip: jax.Array,
    B_x: jax.Array,
    B_w1: jax.Array,
    B_w3: jax.Array,
    B_w2: jax.Array,
):
    return _IMPL(A_x, A_Lambda_re, A_Lambda_im, A_B_re, A_B_im, A_C_re, A_C_im, A_log_dt, A_Dskip,
                 B_x, B_w1, B_w3, B_w2)
```

```python
import jax
import jax.numpy as jnp
from jax import lax
import jax.experimental.pallas as pl
import jax.experimental.pallas.tpu as pltpu

F32 = jnp.float32
BF16 = jnp.bfloat16
I32 = jnp.int32
NT = (((1,), (1,)), ((), ()))


def _cmul(ar, ai, br, bi):
    return ar * br - ai * bi, ar * bi + ai * br


def _exp_expm1(a):
    ac = jnp.clip(a, -104.0, 89.0)
    k = jnp.floor(ac * 1.4426950408889634 + 0.5)
    r = (ac - k * 0.693145751953125) - k * 1.42860682030941723212e-6
    p = 1.0 / 40320.0
    for c in (1.0 / 5040.0, 1.0 / 720.0, 1.0 / 120.0, 1.0 / 24.0, 1.0 / 6.0, 0.5):
        p = p * r + c
    p = (p * r) * r + r
    ki = k.astype(I32)
    k1 = ki >> 1
    s1 = pltpu.bitcast((k1 + 127) << 23, F32)
    s2 = pltpu.bitcast((ki - k1 + 127) << 23, F32)
    e = (s1 * (1.0 + p)) * s2
    return e, jnp.where(ki == 0, p, e - 1.0)


def _swiglu(g, u):
    hg = 0.5 * g
    return ((hg * jnp.tanh(hg) + hg) * u).astype(BF16)


def _or_all(vs):
    acc = vs[0]
    for v in vs[1:]:
        acc = acc | v
    return acc


def _pin(lhs, link):
    if link is None:
        return lhs
    blk = pltpu.bitcast(pltpu.bitcast(lhs[0:16, 0:128], I32) | link, BF16)
    top = jnp.concatenate([blk, lhs[0:16, 128:]], axis=1) if lhs.shape[1] > 128 else blk
    return jnp.concatenate([top, lhs[16:, :]], axis=0)


def _pin32(v, link):
    if link is None:
        return v
    blk = pltpu.bitcast(pltpu.bitcast(v[0:8, :], I32) | link, F32)
    return jnp.concatenate([blk, v[8:, :]], axis=0)


def make(T=256, NA=6, ND=4, NBA=3, KA=2, KB=4, RB=32, ORD='S-S-S-S-S----', LP=(1, 1, 1, 1, 1, 1, 1, 1, 0, 0), MID=False):
    S = T // 8
    PITCH = S + 4
    NB = T // RB

    def kernel(x_hbm, lre_hbm, lim_hbm, ldt_hbm, dsk_hbm, bre_hbm, bim_hbm, cre_hbm, cim_hbm,
               w1_hbm, w3_hbm, w2_hbm, o_hbm,
               x_v, par_v, b_v, c_v, w1_v, w3_v, wt_v, w2_v,
               xin_scr, xout_scr, o_v, xn_scr, base_scr, xn0_scr, base0_scr, raw0_scr, dsk_scr,
               lam_scr, pw_scr, cp_scr, carry_scr, raw_scr, zero_scr,
               w_sem):
        L, D = x_v.shape
        P = b_v.shape[1]
        Fh = w2_v.shape[0]
        Fm = (Fh // 128) * 128
        Ft = Fh - Fm
        NG = Fm // 128
        NL = D // 128
        NP = P // 128
        NC = L // T
        i = pl.program_id(0)

        S_PAR, S_X, S_BA, S_BB, S_WA, S_WB, S_W2, S_C, S_O, S_OT = 0, 1, 3, 4, 5, 6, 7, 8, 9, 11

        def x_copy(c):
            return pltpu.make_async_copy(x_hbm.at[0, pl.ds(c * T, T), :], x_v.at[pl.ds(c * T, T), :],
                                         w_sem.at[S_X + c % 2])

        def o_copy(c):
            return pltpu.make_async_copy(o_v.at[c % 2], o_hbm.at[0, pl.ds(c * T, T), :], w_sem.at[S_O + c % 2])

        def o_tile_copy(j):
            c = NC - 1
            cs = pl.ds(128 * j, 128)
            return pltpu.make_async_copy(o_v.at[c % 2, :, cs], o_hbm.at[0, pl.ds(c * T, T), cs], w_sem.at[S_OT])

        cps = {}
        def add(name, sem, src, dst):
            cps.setdefault(name, []).append(pltpu.make_async_copy(src, dst, w_sem.at[sem]))
        for k, r in enumerate((dsk_hbm, lre_hbm, lim_hbm, ldt_hbm)):
            add('par', S_PAR, r, par_v.at[k])
        PA = NBA * 128
        add('ba', S_BA, bre_hbm.at[pl.ds(0, PA), :], b_v.at[0, pl.ds(0, PA), :])
        add('bb', S_BB, bre_hbm.at[pl.ds(PA, P - PA), :], b_v.at[0, pl.ds(PA, P - PA), :])
        add('bb', S_BB, bim_hbm, b_v.at[1])
        FA = NA * 128
        add('wa', S_WA, w1_hbm.at[pl.ds(0, FA), :], w1_v.at[pl.ds(0, FA), :])
        add('wa', S_WA, w3_hbm.at[pl.ds(0, FA), :], w3_v.at[pl.ds(0, FA), :])
        add('wb', S_WB, w1_hbm.at[pl.ds(FA, Fm - FA), :], w1_v.at[pl.ds(FA, Fm - FA), :])
        add('wb', S_WB, w3_hbm.at[pl.ds(FA, Fm - FA), :], w3_v.at[pl.ds(FA, Fm - FA), :])
        add('wb', S_WB, w1_hbm.at[pl.ds(Fm, Ft), :], wt_v.at[pl.ds(0, Ft), :])
        add('wb', S_WB, w3_hbm.at[pl.ds(Fm, Ft), :], wt_v.at[pl.ds(Ft, Ft), :])
        add('w2', S_W2, w2_hbm, w2_v)
        add('c', S_C, cre_hbm, c_v.at[0])
        add('c', S_C, cim_hbm, c_v.at[1])

        def wait(name):
            for cp in cps[name]:
                cp.wait()

        def ln_stage(c):
            start = c * T if isinstance(c, int) else pl.multiple_of(c * T, T)
            xf = x_v[pl.ds(start, T), :].astype(F32)
            for j in range(NL):
                for s in range(8):
                    xin_scr[j, pl.ds(PITCH * s, S), :] = xf[S * s:S * (s + 1), 128 * j:128 * (j + 1)]

        def ln_block(r):
            ts = range(r * RB // 8, (r + 1) * RB // 8)
            xp = jnp.concatenate(
                [jnp.concatenate([xin_scr[j, pl.ds(t, 8, stride=PITCH), :] for t in ts], axis=0)
                 for j in range(NL)], axis=1)
            mean = jnp.sum(xp, axis=-1, keepdims=True) * (1.0 / D)
            xc = xp - mean
            var = jnp.sum(xc * xc, axis=-1, keepdims=True) * (1.0 / D)
            m_b = mean.astype(BF16).astype(F32)
            v_b = var.astype(BF16).astype(F32)
            sd = jnp.sqrt((v_b + 1e-5).astype(BF16).astype(F32)).astype(BF16).astype(F32)
            xn = ((xp - m_b) * (1.0 / sd)).astype(BF16)
            base = xp + xn.astype(F32) * dsk_scr[0:1, :]
            bi = pltpu.bitcast(base, I32)
            link = _or_all([bi[8 * a:8 * a + 8, 128 * j:128 * (j + 1)] for a in range(RB // 8) for j in range(NL)])
            return xn, base, link & zero_scr[...]

        def ln_full(c, xn_dst, base_dst):
            ln_stage(c)
            for r in range(NB):
                xn, base, _ = ln_block(r)
                xn_dst[r * RB:(r + 1) * RB, :] = xn
                base_dst[r * RB:(r + 1) * RB, :] = base

        def row_table(v):
            return jnp.concatenate([jnp.broadcast_to(v[j:j + 1, :], (8, 128)) for j in range(v.shape[0])], axis=1)

        def prep_params():
            dsk_scr[...] = row_table(par_v[0].astype(F32))
            lr = par_v[1].astype(F32)
            li = par_v[2].astype(F32)
            dt = _exp_expm1(par_v[3].astype(F32))[0].astype(BF16).astype(F32)
            a = dt * lr
            b = dt * li
            mag, magm1 = _exp_expm1(a)
            cb = jnp.cos(b)
            sh = jnp.sin(0.5 * b)
            lbr = mag * cb
            lbi = mag * jnp.sin(b)
            nr = magm1 * cb - 2.0 * (sh * sh)
            ni = lbi
            big = jnp.abs(lr) >= jnp.abs(li)
            r1 = li / lr
            d1 = lr + li * r1
            r2 = lr / li
            d2 = lr * r2 + li
            cr = jnp.where(big, (nr + ni * r1) / d1, (nr * r2 + ni) / d2)
            ci = jnp.where(big, (ni - nr * r1) / d1, (ni * r2 - nr) / d2)
            lam_scr[0] = row_table(lbr)
            lam_scr[1] = row_table(lbi)
            lam_scr[2] = row_table(2.0 * cr)
            lam_scr[3] = row_table(2.0 * ci)
            pr, pi = lbr, lbi
            n = 1
            while n < S:
                pr, pi = _cmul(pr, pi, pr, pi)
                n *= 2
            for k in range(3):
                pw_scr[2 * k] = row_table(pr)
                pw_scr[2 * k + 1] = row_table(pi)
                pr, pi = _cmul(pr, pi, pr, pi)
            carry_scr[...] = jnp.zeros(carry_scr.shape, F32)
            zero_scr[...] = jnp.zeros(zero_scr.shape, I32)

        def prep_c():
            cr = lam_scr[2, 0:1, :]
            ci = lam_scr[3, 0:1, :]
            RC = 64
            for r in range(0, D, RC):
                c_r = c_v[0, r:r + RC, :].astype(F32)
                c_i = c_v[1, r:r + RC, :].astype(F32)
                cp_scr[r:r + RC, :P] = (c_r * cr - c_i * ci).astype(BF16)
                cp_scr[r:r + RC, P:] = (-(c_r * ci) - c_i * cr).astype(BF16)

        def scan_tile(j, raw):
            sub = lax.broadcasted_iota(I32, (8, 128), 0)
            cr_ = slice(128 * j, 128 * (j + 1))
            ci_ = slice(P + 128 * j, P + 128 * (j + 1))
            lbr = lam_scr[0, :, cr_]
            lbi = lam_scr[1, :, cr_]
            er = raw[0:8, cr_]
            ei = raw[0:8, ci_]
            for t in range(1, S):
                ur = raw[8 * t:8 * t + 8, cr_]
                ui = raw[8 * t:8 * t + 8, ci_]
                er, ei = (lbr * er - lbi * ei) + ur, (lbr * ei + lbi * er) + ui
            vr = pltpu.roll(jnp.where(sub == 7, carry_scr[0, :, cr_], er), 1, 0)
            vi = pltpu.roll(jnp.where(sub == 7, carry_scr[1, :, cr_], ei), 1, 0)
            for k in range(3):
                sh = 1 << k
                ar = pw_scr[2 * k, :, cr_]
                ai = pw_scr[2 * k + 1, :, cr_]
                sr = pltpu.roll(vr, sh, 0)
                si = pltpu.roll(vi, sh, 0)
                tr, ti = _cmul(ar, ai, sr, si)
                msk = sub >= sh
                vr = vr + jnp.where(msk, tr, 0.0)
                vi = vi + jnp.where(msk, ti, 0.0)
            hr, hi = vr, vi
            prs, pis = [], []
            for t2 in range(S // 2):
                outs = []
                for t in (2 * t2, 2 * t2 + 1):
                    ur = raw[8 * t:8 * t + 8, cr_]
                    ui = raw[8 * t:8 * t + 8, ci_]
                    hr, hi = (lbr * hr - lbi * hi) + ur, (lbr * hi + lbi * hr) + ui
                    outs.append((hr, hi))
                prs.append(jnp.concatenate([outs[0][0], outs[1][0]], axis=0).astype(BF16))
                pis.append(jnp.concatenate([outs[0][1], outs[1][1]], axis=0).astype(BF16))
            carry_scr[0, :, cr_] = hr
            carry_scr[1, :, cr_] = hi
            link = _or_all([pltpu.bitcast(v, I32) for pr_pi in zip(prs, pis) for v in pr_pi])
            return jnp.concatenate(prs, axis=0), jnp.concatenate(pis, axis=0), link & zero_scr[...]

        def up_stage(xn_ref, raw, first):
            if first:
                wait('wa')
            xn = xn_ref[...]
            hs, g_re, g_im = [], [], []
            for gi in range(NG):
                if first and gi == NA:
                    first()
                    wait('wb')
                    xn = xn_ref[...]
                lk = None
                if ORD[gi] == 'S' and len(g_re) < NP:
                    gr, gim, lk = scan_tile(len(g_re), raw)
                    g_re.append(gr)
                    g_im.append(gim)
                rs = slice(128 * gi, 128 * (gi + 1))
                gate = lax.dot_general(xn, w1_v[rs, :], NT, preferred_element_type=F32)
                up = lax.dot_general(xn, w3_v[rs, :], NT, preferred_element_type=F32)
                hs.append(_pin(_swiglu(gate, up), lk))
            tail = lax.dot_general(xn, wt_v[...], NT, preferred_element_type=F32)
            ht = _swiglu(tail[:, :Ft], tail[:, Ft:])
            assert len(g_re) == NP
            return jnp.concatenate(hs, axis=1), ht, jnp.concatenate(g_re + g_im, axis=1)

        def write_out(out, c):
            last = isinstance(c, int) and c == NC - 1
            for j in range(NL):
                for t in range(S):
                    xout_scr[j, pl.ds(t, 8, stride=PITCH), :] = out[8 * t:8 * t + 8, 128 * j:128 * (j + 1)]
                for s in range(8):
                    o_v[c % 2, S * s:S * (s + 1), 128 * j:128 * (j + 1)] = xout_scr[j, pl.ds(PITCH * s, S), :]
                if last:
                    o_tile_copy(j).start()
            if not last:
                o_copy(c).start()

        def main(last):
            if not last:
                ln_stage(i + 1)
            h, ht, g = up_stage(xn_scr, raw_scr, None)
            xns, bases = [], []

            def ln_pin(k):
                lk = None
                if not last:
                    for _ in range(LP[k]):
                        if len(xns) < NB:
                            r = len(xns)
                            xb, bb, l2 = ln_block(r)
                            xn_scr[r * RB:(r + 1) * RB, :] = xb
                            xns.append(xb)
                            bases.append(bb)
                            lk = l2 if lk is None else lk | l2
                return lk

            ys = []
            for n in range(NL):
                cs = slice(128 * n, 128 * (n + 1))
                yn = jnp.dot(h, w2_v[:Fm, cs], preferred_element_type=F32)
                yn = _pin32(yn, ln_pin(2 * n))
                yn = yn + jnp.dot(ht, w2_v[Fm:, cs], preferred_element_type=F32)
                yn = yn + lax.dot_general(g, cp_scr[cs, :], NT, preferred_element_type=F32)
                yn = _pin32(yn, ln_pin(2 * n + 1))
                ys.append(yn)
            y = jnp.concatenate(ys, axis=1)
            if not last:
                assert len(xns) == NB
                xn_next = jnp.concatenate(xns, axis=0)
                raw_scr[:, :P] = lax.dot_general(xn_next, b_v[0], NT, preferred_element_type=F32)
                raw_scr[:, P:] = lax.dot_general(xn_next, b_v[1], NT, preferred_element_type=F32)
            out = base_scr[...] + y
            if not last:
                base_scr[...] = jnp.concatenate(bases, axis=0)
            write_out(out, NC - 1 if last else i)

        def first_step():
            for cp in cps['par']:
                cp.start()
            x_copy(0).start()
            x_copy(1).start()
            for n in cps:
                if n != 'par':
                    for cp in cps[n]:
                        cp.start()
            wait('par')
            prep_params()
            x_copy(0).wait()
            x_copy(2).start()
            ln_full(0, xn0_scr, base0_scr)
            x_copy(1).wait()
            ln_full(1, xn_scr, base_scr)
            PB = PA - 128
            PL = P - 128
            K1, K2 = KA * 128, KB * 128

            def bdot(xr, k0, k1, w, n0, n1):
                return lax.dot_general(xr[:, k0:k1], b_v[w, n0:n1, k0:k1], NT, preferred_element_type=F32)

            wait('ba')
            raw0_scr[:, :PA] = bdot(xn0_scr, 0, D, 0, 0, PA)
            raw_scr[:, :PB] = bdot(xn_scr, 0, D, 0, 0, PB)
            raw_scr[:, PB:PA] = bdot(xn_scr, 0, K1, 0, PB, PA)
            wait('bb')
            raw0_scr[:, PA:P] = bdot(xn0_scr, 0, D, 0, PA, P)
            raw0_scr[:, P:] = bdot(xn0_scr, 0, D, 1, 0, P)
            raw_scr[:, PA:P] = bdot(xn_scr, 0, D, 0, PA, P)
            raw_scr[:, P:P + PL] = bdot(xn_scr, 0, D, 1, 0, PL)
            raw_scr[:, PB:PA] += bdot(xn_scr, K1, D, 0, PB, PA)

            def extra_a():
                raw_scr[:, P + PL:] = bdot(xn_scr, 0, K2, 1, PL, P)

            h, ht, g = up_stage(xn0_scr, raw0_scr, extra_a)
            if K2 < D:
                raw_scr[:, P + PL:] += bdot(xn_scr, K2, D, 1, PL, P)
            wait('w2')
            ys = []
            for n in range(NL):
                if n == ND:
                    wait('c')
                    prep_c()
                cs = slice(128 * n, 128 * (n + 1))
                yn = jnp.dot(h, w2_v[:Fm, cs], preferred_element_type=F32)
                yn = yn + jnp.dot(ht, w2_v[Fm:, cs], preferred_element_type=F32)
                ys.append(yn)
            y = jnp.concatenate(ys, axis=1)
            y = y + lax.dot_general(g, cp_scr[...], NT, preferred_element_type=F32)
            write_out(base0_scr[...] + y, 0)

        @pl.when(i == 0)
        def _():
            first_step()
            x_copy(2).wait()

        @pl.when(jnp.logical_and(i > 0, i < NC - 1))
        def _():
            @pl.when(i + 2 < NC)
            def _():
                x_copy(i + 2).start()
            main(False)

            @pl.when(i + 2 < NC)
            def _():
                x_copy(i + 2).wait()
            o_copy(i - 1).wait()

        @pl.when(i == NC - 1)
        def _():
            main(True)
            o_copy(NC - 2).wait()
            for j in range(NL):
                o_tile_copy(j).wait()

    @jax.jit
    def f(A_x, A_Lambda_re, A_Lambda_im, A_B_re, A_B_im, A_C_re, A_C_im, A_log_dt, A_Dskip, B_x, B_w1, B_w3, B_w2):
        Bsz, L, D = A_x.shape
        P = A_Lambda_re.shape[0]
        Fh = B_w1.shape[1]
        Ft = Fh % 128
        Fm = Fh - Ft
        NC = L // T
        vec = lambda a: a.reshape(-1, 128)
        args = (A_x, vec(A_Lambda_re), vec(A_Lambda_im), vec(A_log_dt), vec(A_Dskip),
                A_B_re, A_B_im, A_C_re, A_C_im, B_w1.T, B_w3.T, B_w2)
        return pl.pallas_call(
            kernel,
            grid=(NC,),
            in_specs=[pl.BlockSpec(memory_space=pl.ANY)] * len(args),
            out_specs=pl.BlockSpec(memory_space=pl.ANY),
            out_shape=jax.ShapeDtypeStruct((Bsz, L, D), F32),
            scratch_shapes=[
                pltpu.VMEM((L, D), BF16),
                pltpu.VMEM((4, P // 128, 128), BF16),
                pltpu.VMEM((2, P, D), BF16),
                pltpu.VMEM((2, D, P), BF16),
                pltpu.VMEM((Fm, D), BF16),
                pltpu.VMEM((Fm, D), BF16),
                pltpu.VMEM((2 * Ft, D), BF16),
                pltpu.VMEM((Fh, D), BF16),
                pltpu.VMEM((D // 128, 8 * PITCH, 128), F32),
                pltpu.VMEM((D // 128, 8 * PITCH, 128), F32),
                pltpu.VMEM((2, T, D), F32),
                pltpu.VMEM((T, D), BF16),
                pltpu.VMEM((T, D), F32),
                pltpu.VMEM((T, D), BF16),
                pltpu.VMEM((T, D), F32),
                pltpu.VMEM((T, 2 * P), F32),
                pltpu.VMEM((8, D), F32),
                pltpu.VMEM((4, 8, P), F32),
                pltpu.VMEM((6, 8, P), F32),
                pltpu.VMEM((D, 2 * P), BF16),
                pltpu.VMEM((2, 8, P), F32),
                pltpu.VMEM((T, 2 * P), F32),
                pltpu.VMEM((8, 128), I32),
                pltpu.SemaphoreType.DMA((12,)),
            ],
            compiler_params=pltpu.CompilerParams(dimension_semantics=("arbitrary",),
                                                 vmem_limit_bytes=100 * 1024 * 1024),
        )(*args)
    return f


_IMPL = make()


@jax.jit
def pallas_parallel_sum__ssm_conv_s5__glu_gated_swiglu__prompt_kernel(
    A_x: jax.Array,
    A_Lambda_re: jax.Array,
    A_Lambda_im: jax.Array,
    A_B_re: jax.Array,
    A_B_im: jax.Array,
    A_C_re: jax.Array,
    A_C_im: jax.Array,
    A_log_dt: jax.Array,
    A_Dskip: jax.Array,
    B_x: jax.Array,
    B_w1: jax.Array,
    B_w3: jax.Array,
    B_w2: jax.Array,
):
    return _IMPL(A_x, A_Lambda_re, A_Lambda_im, A_B_re, A_B_im, A_C_re, A_C_im, A_log_dt, A_Dskip,
                 B_x, B_w1, B_w3, B_w2)
```

```python
import jax
import jax.numpy as jnp
from jax import lax
import jax.experimental.pallas as pl
import jax.experimental.pallas.tpu as pltpu

F32 = jnp.float32
BF16 = jnp.bfloat16
I32 = jnp.int32
NT = (((1,), (1,)), ((), ()))

T = 256
S = T // 8
PITCH = S + 4
RB = 32
NB = T // RB
NBA, KA, KB, NA, ND = 4, 2, 4, 10, 2
ORD_FIRST = '-S-S-S-S-S---'
ORD_MAIN = 'S-S-S-S-S----'
LN_PINS = (1, 1, 1, 1, 1, 1, 1, 1, 0, 0)
S_PAR, S_X, S_BA, S_BB, S_WA, S_WB, S_C, S_O, N_SEM = 0, 1, 3, 4, 5, 6, 7, 8, 10


def _cmul(ar, ai, br, bi):
    return ar * br - ai * bi, ar * bi + ai * br


def _exp_expm1(a):
    ac = jnp.clip(a, -104.0, 89.0)
    k = jnp.floor(ac * 1.4426950408889634 + 0.5)
    r = (ac - k * 0.693145751953125) - k * 1.42860682030941723212e-6
    p = 1.0 / 40320.0
    for c in (1.0 / 5040.0, 1.0 / 720.0, 1.0 / 120.0, 1.0 / 24.0, 1.0 / 6.0, 0.5):
        p = p * r + c
    p = (p * r) * r + r
    ki = k.astype(I32)
    k1 = ki >> 1
    s1 = pltpu.bitcast((k1 + 127) << 23, F32)
    s2 = pltpu.bitcast((ki - k1 + 127) << 23, F32)
    e = (s1 * (1.0 + p)) * s2
    return e, jnp.where(ki == 0, p, e - 1.0)


def _swiglu(g, u):
    hg = 0.5 * g
    return ((hg * jnp.tanh(hg) + hg) * u).astype(BF16)


def _or_all(vs):
    acc = vs[0]
    for v in vs[1:]:
        acc = acc | v
    return acc


def _pin(v, link):
    if link is None:
        return v
    blk = pltpu.bitcast(pltpu.bitcast(v[0:16, :], I32) | link, BF16)
    return jnp.concatenate([blk, v[16:, :]], axis=0)


def _pin32(v, link):
    if link is None:
        return v
    blk = pltpu.bitcast(pltpu.bitcast(v[0:8, :], I32) | link, F32)
    return jnp.concatenate([blk, v[8:, :]], axis=0)


def _kernel(x_hbm, lre_hbm, lim_hbm, ldt_hbm, dsk_hbm, bre_hbm, bim_hbm, cre_hbm, cim_hbm,
            w1_hbm, w3_hbm, w2_hbm, o_hbm,
            x_v, par_v, b_v, c_v, w1_v, w3_v, wt_v, w2_v,
            xin_scr, xout_scr, o_v, xn_scr, base_scr, raw_scr, xn0_scr, base0_scr, raw0_scr,
            dsk_scr, lam_scr, pw_scr, cp_scr, carry_scr, zero_scr, w1t_scr, sem):
    L, D = x_v.shape
    P = b_v.shape[1]
    Fh = w2_v.shape[0]
    Fm = (Fh // 128) * 128
    Ft = Fh - Fm
    NG, NL, NP, NC = Fm // 128, D // 128, P // 128, L // T
    i = pl.program_id(0)

    def x_copy(c, slot=None):
        slot = S_X + (c & 1) if slot is None else slot
        return pltpu.make_async_copy(x_hbm.at[0, pl.ds(c * T, T), :], x_v.at[pl.ds(c * T, T), :], sem.at[slot])

    def o_copy(c):
        return pltpu.make_async_copy(o_v.at[c & 1], o_hbm.at[0, pl.ds(c * T, T), :], sem.at[S_O + (c & 1)])

    def o_tile_copy(c, j):
        cs = pl.ds(128 * j, 128)
        return pltpu.make_async_copy(o_v.at[c & 1, :, cs], o_hbm.at[0, pl.ds(c * T, T), cs],
                                     sem.at[S_O + (c & 1)])

    def weight_copies():
        cps = {}

        def add(name, slot, src, dst):
            cps.setdefault(name, []).append(pltpu.make_async_copy(src, dst, sem.at[slot]))

        for k, r in enumerate((dsk_hbm, lre_hbm, lim_hbm, ldt_hbm)):
            add('par', S_PAR, r, par_v.at[k])
        PA, FA = NBA * 128, NA * 128
        add('ba', S_BA, bre_hbm.at[pl.ds(0, PA), :], b_v.at[0, pl.ds(0, PA), :])
        cps['bb'] = [x_copy(2, S_BB)]
        add('bb', S_BB, bre_hbm.at[pl.ds(PA, P - PA), :], b_v.at[0, pl.ds(PA, P - PA), :])
        add('bb', S_BB, bim_hbm, b_v.at[1])
        add('wa', S_WA, w1_hbm.at[pl.ds(0, FA), :], w1_v.at[pl.ds(0, FA), :])
        add('wa', S_WA, w3_hbm.at[pl.ds(0, FA), :], w3_v.at[pl.ds(0, FA), :])
        add('wb', S_WB, w1_hbm.at[pl.ds(FA, Fm - FA), :], w1_v.at[pl.ds(FA, Fm - FA), :])
        add('wb', S_WB, w3_hbm.at[pl.ds(FA, Fm - FA), :], w3_v.at[pl.ds(FA, Fm - FA), :])
        add('wb', S_WB, w1_hbm.at[pl.ds(Fm, Ft), :], wt_v.at[pl.ds(0, Ft), :])
        add('wb', S_WB, w3_hbm.at[pl.ds(Fm, Ft), :], wt_v.at[pl.ds(Ft, Ft), :])
        add('wb', S_WB, w2_hbm, w2_v)
        add('c', S_C, cre_hbm, c_v.at[0])
        add('c', S_C, cim_hbm, c_v.at[1])
        return cps

    def ln_stage(c):
        start = c * T if isinstance(c, int) else pl.multiple_of(c * T, T)
        xf = x_v[pl.ds(start, T), :].astype(F32)
        for j in range(NL):
            for s in range(8):
                xin_scr[j, pl.ds(PITCH * s, S), :] = xf[S * s:S * (s + 1), 128 * j:128 * (j + 1)]

    def ln_block(r):
        ts = range(r * RB // 8, (r + 1) * RB // 8)
        xp = jnp.concatenate(
            [jnp.concatenate([xin_scr[j, pl.ds(t, 8, stride=PITCH), :] for t in ts], axis=0)
             for j in range(NL)], axis=1)
        mean = jnp.sum(xp, axis=-1, keepdims=True) * (1.0 / D)
        xc = xp - mean
        var = jnp.sum(xc * xc, axis=-1, keepdims=True) * (1.0 / D)
        m_b = mean.astype(BF16).astype(F32)
        v_b = var.astype(BF16).astype(F32)
        sd = jnp.sqrt((v_b + 1e-5).astype(BF16).astype(F32)).astype(BF16).astype(F32)
        xn = ((xp - m_b) * (1.0 / sd)).astype(BF16)
        base = xp + xn.astype(F32) * dsk_scr[0:1, :]
        bi = pltpu.bitcast(base, I32)
        link = _or_all([bi[8 * a:8 * a + 8, 128 * j:128 * (j + 1)] for a in range(RB // 8) for j in range(NL)])
        return xn, base, link & zero_scr[...]

    def ln_full(c, xn_dst, base_dst):
        ln_stage(c)
        for r in range(NB):
            xn, base, _ = ln_block(r)
            xn_dst[r * RB:(r + 1) * RB, :] = xn
            base_dst[r * RB:(r + 1) * RB, :] = base

    def row_table(v):
        return jnp.concatenate([jnp.broadcast_to(v[j:j + 1, :], (8, 128)) for j in range(v.shape[0])], axis=1)

    def prep_params():
        dsk_scr[...] = row_table(par_v[0].astype(F32))
        lr = par_v[1].astype(F32)
        li = par_v[2].astype(F32)
        dt = _exp_expm1(par_v[3].astype(F32))[0].astype(BF16).astype(F32)
        a = dt * lr
        b = dt * li
        mag, magm1 = _exp_expm1(a)
        cb = jnp.cos(b)
        sh = jnp.sin(0.5 * b)
        lbr = mag * cb
        lbi = mag * jnp.sin(b)
        nr = magm1 * cb - 2.0 * (sh * sh)
        ni = lbi
        big = jnp.abs(lr) >= jnp.abs(li)
        r1 = li / lr
        d1 = lr + li * r1
        r2 = lr / li
        d2 = lr * r2 + li
        cr = jnp.where(big, (nr + ni * r1) / d1, (nr * r2 + ni) / d2)
        ci = jnp.where(big, (ni - nr * r1) / d1, (ni * r2 - nr) / d2)
        lam_scr[0] = row_table(lbr)
        lam_scr[1] = row_table(lbi)
        lam_scr[2] = row_table(2.0 * cr)
        lam_scr[3] = row_table(2.0 * ci)
        pr, pi = lbr, lbi
        n = 1
        while n < S:
            pr, pi = _cmul(pr, pi, pr, pi)
            n *= 2
        for k in range(3):
            pw_scr[2 * k] = row_table(pr)
            pw_scr[2 * k + 1] = row_table(pi)
            pr, pi = _cmul(pr, pi, pr, pi)
        carry_scr[...] = jnp.zeros(carry_scr.shape, F32)
        zero_scr[...] = jnp.zeros(zero_scr.shape, I32)

    def prep_c():
        cr = lam_scr[2, 0:1, :]
        ci = lam_scr[3, 0:1, :]
        RC = 64
        for r in range(0, D, RC):
            c_r = c_v[0, r:r + RC, :].astype(F32)
            c_i = c_v[1, r:r + RC, :].astype(F32)
            cp_scr[r:r + RC, :P] = (c_r * cr - c_i * ci).astype(BF16)
            cp_scr[r:r + RC, P:] = (-(c_r * ci) - c_i * cr).astype(BF16)

    def scan_tile(j, raw):
        sub = lax.broadcasted_iota(I32, (8, 128), 0)
        cr_ = slice(128 * j, 128 * (j + 1))
        ci_ = slice(P + 128 * j, P + 128 * (j + 1))
        lbr = lam_scr[0, :, cr_]
        lbi = lam_scr[1, :, cr_]
        er = raw[0:8, cr_]
        ei = raw[0:8, ci_]
        for t in range(1, S):
            ur = raw[8 * t:8 * t + 8, cr_]
            ui = raw[8 * t:8 * t + 8, ci_]
            er, ei = (lbr * er - lbi * ei) + ur, (lbr * ei + lbi * er) + ui
        vr = pltpu.roll(jnp.where(sub == 7, carry_scr[0, :, cr_], er), 1, 0)
        vi = pltpu.roll(jnp.where(sub == 7, carry_scr[1, :, cr_], ei), 1, 0)
        for k in range(3):
            sh = 1 << k
            tr, ti = _cmul(pw_scr[2 * k, :, cr_], pw_scr[2 * k + 1, :, cr_],
                           pltpu.roll(vr, sh, 0), pltpu.roll(vi, sh, 0))
            msk = sub >= sh
            vr = vr + jnp.where(msk, tr, 0.0)
            vi = vi + jnp.where(msk, ti, 0.0)
        hr, hi = vr, vi
        prs, pis = [], []
        for t2 in range(S // 2):
            outs = []
            for t in (2 * t2, 2 * t2 + 1):
                ur = raw[8 * t:8 * t + 8, cr_]
                ui = raw[8 * t:8 * t + 8, ci_]
                hr, hi = (lbr * hr - lbi * hi) + ur, (lbr * hi + lbi * hr) + ui
                outs.append((hr, hi))
            prs.append(jnp.concatenate([outs[0][0], outs[1][0]], axis=0).astype(BF16))
            pis.append(jnp.concatenate([outs[0][1], outs[1][1]], axis=0).astype(BF16))
        carry_scr[0, :, cr_] = hr
        carry_scr[1, :, cr_] = hi
        link = _or_all([pltpu.bitcast(v, I32) for pr_pi in zip(prs, pis) for v in pr_pi])
        return jnp.concatenate(prs, axis=0), jnp.concatenate(pis, axis=0), link & zero_scr[...]

    def up_stage(xn_ref, raw, wait):
        order = ORD_FIRST if wait else ORD_MAIN
        if wait:
            wait('wa')
        xn = xn_ref[...]
        hs, g_re, g_im = [], [], []
        for gi in range(NG):
            if wait and gi == NA:
                wait('wb')
                xn = xn_ref[...]
            lk = None
            if order[gi] == 'S':
                gr, gim, lk = scan_tile(len(g_re), raw)
                g_re.append(gr)
                g_im.append(gim)
            rs = slice(128 * gi, 128 * (gi + 1))
            if gi == 0 and not wait:
                gate = jnp.dot(xn, w1t_scr[...], preferred_element_type=F32)
            else:
                gate = lax.dot_general(xn, w1_v[rs, :], NT, preferred_element_type=F32)
            up = lax.dot_general(xn, w3_v[rs, :], NT, preferred_element_type=F32)
            hs.append(_pin(_swiglu(gate, up), lk))
        tail = lax.dot_general(xn, wt_v[...], NT, preferred_element_type=F32)
        ht = _swiglu(tail[:, :Ft], tail[:, Ft:])
        assert len(g_re) == NP
        return jnp.concatenate(hs, axis=1), ht, jnp.concatenate(g_re + g_im, axis=1)

    def write_out(out, c, tiles):
        for j in range(NL):
            for t in range(S):
                xout_scr[j, pl.ds(t, 8, stride=PITCH), :] = out[8 * t:8 * t + 8, 128 * j:128 * (j + 1)]
            for s in range(8):
                o_v[c & 1, S * s:S * (s + 1), 128 * j:128 * (j + 1)] = xout_scr[j, pl.ds(PITCH * s, S), :]
            if tiles:
                o_tile_copy(c, j).start()
        if not tiles:
            o_copy(c).start()

    def main(last):
        p = i & 1
        xn_p, base_p, raw_p = xn_scr.at[p], base_scr.at[p], raw_scr.at[p]
        if not last:
            ln_stage(i + 2)
        h, ht, g = up_stage(xn_p, raw_p, None)
        xns, bases = [], []

        def ln_pin(k):
            lk = None
            for _ in range(0 if last else LN_PINS[k]):
                r = len(xns)
                xb, bb, l2 = ln_block(r)
                xn_p[r * RB:(r + 1) * RB, :] = xb
                xns.append(xb)
                bases.append(bb)
                lk = l2 if lk is None else lk | l2
            return lk

        ys = []
        for n in range(NL):
            cs = slice(128 * n, 128 * (n + 1))
            yn = jnp.dot(h, w2_v[:Fm, cs], preferred_element_type=F32)
            yn = _pin32(yn, ln_pin(2 * n))
            yn = yn + jnp.dot(ht, w2_v[Fm:, cs], preferred_element_type=F32)
            yn = yn + lax.dot_general(g, cp_scr[cs, :], NT, preferred_element_type=F32)
            yn = _pin32(yn, ln_pin(2 * n + 1))
            ys.append(yn)
        y = jnp.concatenate(ys, axis=1)
        if not last:
            assert len(xns) == NB
            xn_next = jnp.concatenate(xns, axis=0)
            raw_p[:, :P] = lax.dot_general(xn_next, b_v[0], NT, preferred_element_type=F32)
            raw_p[:, P:] = lax.dot_general(xn_next, b_v[1], NT, preferred_element_type=F32)
        out = base_p[...] + y
        if not last:
            base_p[...] = jnp.concatenate(bases, axis=0)
        write_out(out, i, last)

    def first_step():
        cps = weight_copies()

        def wait(name):
            for cp in cps[name]:
                cp.wait()

        for cp in cps['par']:
            cp.start()
        x_copy(0).start()
        x_copy(1).start()
        for name in cps:
            if name != 'par':
                for cp in cps[name]:
                    cp.start()
        wait('par')
        prep_params()
        x_copy(0).wait()
        ln_full(0, xn0_scr, base0_scr)
        x_copy(1).wait()
        x_copy(3).start()
        xn1, base1, raw1 = xn_scr.at[1], base_scr.at[1], raw_scr.at[1]
        xn2, base2, raw2 = xn_scr.at[0], base_scr.at[0], raw_scr.at[0]
        ln_full(1, xn1, base1)

        PA = NBA * 128
        PB, PL = PA - 128, P - 128
        K1, K2 = KA * 128, KB * 128

        def bdot(xr, k0, k1, w, n0, n1):
            return lax.dot_general(xr[:, k0:k1], b_v[w, n0:n1, k0:k1], NT, preferred_element_type=F32)

        wait('ba')
        raw0_scr[:, :PA] = bdot(xn0_scr, 0, D, 0, 0, PA)
        raw1[:, :PB] = bdot(xn1, 0, D, 0, 0, PB)
        raw1[:, PB:PA] = bdot(xn1, 0, K1, 0, PB, PA)
        wait('bb')
        ln_stage(2)
        xns = []

        def ln2():
            if len(xns) == NB:
                return None
            r = len(xns)
            xb, bb, lk = ln_block(r)
            xn2[r * RB:(r + 1) * RB, :] = xb
            base2[r * RB:(r + 1) * RB, :] = bb
            xns.append(xb)
            return lk

        jobs = [(xn0_scr, raw0_scr, 0, n) for n in range(NBA, NP)] + [(xn0_scr, raw0_scr, 1, n) for n in range(NP)]
        jobs += [(xn1, raw1, 0, n) for n in range(NBA, NP)] + [(xn1, raw1, 1, n) for n in range(NP - 1)]
        for q, (xr, rw, w, n) in enumerate(jobs):
            lk = ln2() if q >= 1 else None
            res = bdot(xr, 0, D, w, 128 * n, 128 * (n + 1))
            rw[:, w * P + 128 * n:w * P + 128 * (n + 1)] = _pin32(res, lk)
        raw1[:, PB:PA] += bdot(xn1, K1, D, 0, PB, PA)
        raw1[:, P + PL:] = bdot(xn1, 0, K2, 1, PL, P)
        assert len(xns) == NB
        xx = jnp.concatenate(xns, axis=0)
        raw2[:, :P] = lax.dot_general(xx, b_v[0], NT, preferred_element_type=F32)
        raw2[:, P:] = lax.dot_general(xx, b_v[1], NT, preferred_element_type=F32)

        h, ht, g = up_stage(xn0_scr, raw0_scr, wait)
        raw1[:, P + PL:] += bdot(xn1, K2, D, 1, PL, P)
        w1t_scr[...] = w1_v[0:128, :].astype(F32).T.astype(BF16)
        ys = []
        for n in range(NL):
            if n == ND:
                wait('c')
                prep_c()
            cs = slice(128 * n, 128 * (n + 1))
            yn = jnp.dot(h, w2_v[:Fm, cs], preferred_element_type=F32)
            yn = yn + jnp.dot(ht, w2_v[Fm:, cs], preferred_element_type=F32)
            ys.append(yn)
        y = jnp.concatenate(ys, axis=1)
        y = y + lax.dot_general(g, cp_scr[...], NT, preferred_element_type=F32)
        write_out(base0_scr[...] + y, 0, False)

    @pl.when(i == 0)
    def _():
        first_step()
        x_copy(3).wait()

    @pl.when(jnp.logical_and(i > 0, i < NC - 2))
    def _():
        more_x = i + 3 < NC
        x_next = x_copy(jnp.minimum(i + 3, NC - 1))
        o_prev = o_copy(i - 1)

        @pl.when(more_x)
        def _():
            x_next.start()
        main(False)

        @pl.when(more_x)
        def _():
            x_next.wait()
        o_prev.wait()

    @pl.when(i >= NC - 2)
    def _():
        o_prev = o_copy(i - 1)
        main(True)
        o_prev.wait()

        @pl.when(i == NC - 1)
        def _():
            o_copy(NC - 1).wait()


@jax.jit
def pallas_parallel_sum__ssm_conv_s5__glu_gated_swiglu__prompt_kernel(
    A_x: jax.Array,
    A_Lambda_re: jax.Array,
    A_Lambda_im: jax.Array,
    A_B_re: jax.Array,
    A_B_im: jax.Array,
    A_C_re: jax.Array,
    A_C_im: jax.Array,
    A_log_dt: jax.Array,
    A_Dskip: jax.Array,
    B_x: jax.Array,
    B_w1: jax.Array,
    B_w3: jax.Array,
    B_w2: jax.Array,
):
    del B_x
    Bsz, L, D = A_x.shape
    P = A_Lambda_re.shape[0]
    Fh = B_w1.shape[1]
    Ft = Fh % 128
    Fm = Fh - Ft
    NC = L // T
    assert Bsz == 1 and L % T == 0 and NC >= 4 and D % 128 == 0 and P == D and Ft == 64
    assert Fm // 128 == len(ORD_MAIN) and P // 128 == ORD_MAIN.count('S') and 2 * (D // 128) == len(LN_PINS)
    vec = lambda a: a.reshape(-1, 128)
    args = (A_x, vec(A_Lambda_re), vec(A_Lambda_im), vec(A_log_dt), vec(A_Dskip),
            A_B_re, A_B_im, A_C_re, A_C_im, B_w1.T, B_w3.T, B_w2)
    return pl.pallas_call(
        _kernel,
        grid=(NC,),
        in_specs=[pl.BlockSpec(memory_space=pl.ANY)] * len(args),
        out_specs=pl.BlockSpec(memory_space=pl.ANY),
        out_shape=jax.ShapeDtypeStruct((Bsz, L, D), F32),
        scratch_shapes=[
            pltpu.VMEM((L, D), BF16),
            pltpu.VMEM((4, P // 128, 128), BF16),
            pltpu.VMEM((2, P, D), BF16),
            pltpu.VMEM((2, D, P), BF16),
            pltpu.VMEM((Fm, D), BF16),
            pltpu.VMEM((Fm, D), BF16),
            pltpu.VMEM((2 * Ft, D), BF16),
            pltpu.VMEM((Fh, D), BF16),
            pltpu.VMEM((D // 128, 8 * PITCH, 128), F32),
            pltpu.VMEM((D // 128, 8 * PITCH, 128), F32),
            pltpu.VMEM((2, T, D), F32),
            pltpu.VMEM((2, T, D), BF16),
            pltpu.VMEM((2, T, D), F32),
            pltpu.VMEM((2, T, 2 * P), F32),
            pltpu.VMEM((T, D), BF16),
            pltpu.VMEM((T, D), F32),
            pltpu.VMEM((T, 2 * P), F32),
            pltpu.VMEM((8, D), F32),
            pltpu.VMEM((4, 8, P), F32),
            pltpu.VMEM((6, 8, P), F32),
            pltpu.VMEM((D, 2 * P), BF16),
            pltpu.VMEM((2, 8, P), F32),
            pltpu.VMEM((8, 128), I32),
            pltpu.VMEM((D, 128), BF16),
            pltpu.SemaphoreType.DMA((N_SEM,)),
        ],
        compiler_params=pltpu.CompilerParams(dimension_semantics=("arbitrary",),
                                             vmem_limit_bytes=64 * 1024 * 1024),
    )(*args)
```

```python
import jax
import jax.numpy as jnp
from jax import lax
import jax.experimental.pallas as pl
import jax.experimental.pallas.tpu as pltpu

F32 = jnp.float32
BF16 = jnp.bfloat16
I32 = jnp.int32
NT = (((1,), (1,)), ((), ()))

T = 256
S = T // 8
PITCH = S + 4
RB = 32
NB = T // RB
N0, K0, K1, K2, NA, ND = 3, 3, 4, 4, 10, 2
ORD_FIRST = '-S-S-S-S-S---'
ORD_MAIN = 'S-S-S-S-S----'
LN_PINS = (1, 1, 1, 1, 1, 1, 1, 1, 0, 0)
S_PAR, S_X, S_B0, S_B1, S_B2, S_WA, S_WB, S_C, S_O, N_SEM = 0, 1, 3, 4, 5, 6, 7, 8, 9, 11


def _cmul(ar, ai, br, bi):
    return ar * br - ai * bi, ar * bi + ai * br


def _exp_expm1(a):
    ac = jnp.clip(a, -104.0, 89.0)
    k = jnp.floor(ac * 1.4426950408889634 + 0.5)
    r = (ac - k * 0.693145751953125) - k * 1.42860682030941723212e-6
    p = 1.0 / 40320.0
    for c in (1.0 / 5040.0, 1.0 / 720.0, 1.0 / 120.0, 1.0 / 24.0, 1.0 / 6.0, 0.5):
        p = p * r + c
    p = (p * r) * r + r
    ki = k.astype(I32)
    k1 = ki >> 1
    s1 = pltpu.bitcast((k1 + 127) << 23, F32)
    s2 = pltpu.bitcast((ki - k1 + 127) << 23, F32)
    e = (s1 * (1.0 + p)) * s2
    return e, jnp.where(ki == 0, p, e - 1.0)


def _swiglu(g, u):
    hg = 0.5 * g
    return ((hg * jnp.tanh(hg) + hg) * u).astype(BF16)


def _or_all(vs):
    acc = vs[0]
    for v in vs[1:]:
        acc = acc | v
    return acc


def _pin(v, link):
    if link is None:
        return v
    blk = pltpu.bitcast(pltpu.bitcast(v[0:16, :], I32) | link, BF16)
    return jnp.concatenate([blk, v[16:, :]], axis=0)


def _pin32(v, link):
    if link is None:
        return v
    blk = pltpu.bitcast(pltpu.bitcast(v[0:8, :], I32) | link, F32)
    return jnp.concatenate([blk, v[8:, :]], axis=0)


def _kernel(x_hbm, lre_hbm, lim_hbm, ldt_hbm, dsk_hbm, bre_hbm, bim_hbm, cre_hbm, cim_hbm,
            w1_hbm, w3_hbm, w2_hbm, o_hbm,
            x_v, par_v, b_v, c_v, w1_v, w3_v, wt_v, w2_v,
            xin_scr, xout_scr, o_v, xn_scr, base_scr, raw_scr, xn0_scr, base0_scr, raw0_scr,
            dsk_scr, lam_scr, pw_scr, cp_scr, carry_scr, zero_scr, w1t_scr, sem):
    L, D = x_v.shape
    P = b_v.shape[1]
    Fh = w2_v.shape[0]
    Fm = (Fh // 128) * 128
    Ft = Fh - Fm
    NG, NL, NP, NC = Fm // 128, D // 128, P // 128, L // T
    i = pl.program_id(0)

    def x_copy(c, slot=None):
        slot = S_X + (c & 1) if slot is None else slot
        return pltpu.make_async_copy(x_hbm.at[0, pl.ds(c * T, T), :], x_v.at[pl.ds(c * T, T), :], sem.at[slot])

    def o_copy(c):
        return pltpu.make_async_copy(o_v.at[c & 1], o_hbm.at[0, pl.ds(c * T, T), :], sem.at[S_O + (c & 1)])

    def o_tile_copy(c, j):
        cs = pl.ds(128 * j, 128)
        return pltpu.make_async_copy(o_v.at[c & 1, :, cs], o_hbm.at[0, pl.ds(c * T, T), cs],
                                     sem.at[S_O + (c & 1)])

    def weight_copies():
        cps = {}

        def add(name, slot, src, dst):
            cps.setdefault(name, []).append(pltpu.make_async_copy(src, dst, sem.at[slot]))

        for k, r in enumerate((dsk_hbm, lre_hbm, lim_hbm, ldt_hbm)):
            add('par', S_PAR, r, par_v.at[k])
        PA, FA, WD = N0 * 128, NA * 128, ND * 128
        add('b0', S_B0, bre_hbm.at[pl.ds(0, PA), :], b_v.at[0, pl.ds(0, PA), :])
        cps['b1'] = [x_copy(1, S_B1)]
        add('b1', S_B1, bre_hbm.at[pl.ds(PA, P - PA), :], b_v.at[0, pl.ds(PA, P - PA), :])
        cps['b2'] = [x_copy(2, S_B2)]
        add('b2', S_B2, bim_hbm, b_v.at[1])
        add('wa', S_WA, w1_hbm.at[pl.ds(0, FA), :], w1_v.at[pl.ds(0, FA), :])
        add('wa', S_WA, w3_hbm.at[pl.ds(0, FA), :], w3_v.at[pl.ds(0, FA), :])
        add('wb', S_WB, w1_hbm.at[pl.ds(FA, Fm - FA), :], w1_v.at[pl.ds(FA, Fm - FA), :])
        add('wb', S_WB, w3_hbm.at[pl.ds(FA, Fm - FA), :], w3_v.at[pl.ds(FA, Fm - FA), :])
        add('wb', S_WB, w1_hbm.at[pl.ds(Fm, Ft), :], wt_v.at[pl.ds(0, Ft), :])
        add('wb', S_WB, w3_hbm.at[pl.ds(Fm, Ft), :], wt_v.at[pl.ds(Ft, Ft), :])
        add('wb', S_WB, w2_hbm.at[:, pl.ds(0, WD)], w2_v.at[:, pl.ds(0, WD)])
        add('c', S_C, w2_hbm.at[:, pl.ds(WD, D - WD)], w2_v.at[:, pl.ds(WD, D - WD)])
        add('c', S_C, cre_hbm, c_v.at[0])
        add('c', S_C, cim_hbm, c_v.at[1])
        return cps

    def ln_stage(c):
        start = c * T if isinstance(c, int) else pl.multiple_of(c * T, T)
        xf = x_v[pl.ds(start, T), :].astype(F32)
        for j in range(NL):
            for s in range(8):
                xin_scr[j, pl.ds(PITCH * s, S), :] = xf[S * s:S * (s + 1), 128 * j:128 * (j + 1)]

    def ln_block(r):
        ts = range(r * RB // 8, (r + 1) * RB // 8)
        xp = jnp.concatenate(
            [jnp.concatenate([xin_scr[j, pl.ds(t, 8, stride=PITCH), :] for t in ts], axis=0)
             for j in range(NL)], axis=1)
        mean = jnp.sum(xp, axis=-1, keepdims=True) * (1.0 / D)
        xc = xp - mean
        var = jnp.sum(xc * xc, axis=-1, keepdims=True) * (1.0 / D)
        m_b = mean.astype(BF16).astype(F32)
        v_b = var.astype(BF16).astype(F32)
        sd = jnp.sqrt((v_b + 1e-5).astype(BF16).astype(F32)).astype(BF16).astype(F32)
        xn = ((xp - m_b) * (1.0 / sd)).astype(BF16)
        base = xp + xn.astype(F32) * dsk_scr[0:1, :]
        bi = pltpu.bitcast(base, I32)
        link = _or_all([bi[8 * a:8 * a + 8, 128 * j:128 * (j + 1)] for a in range(RB // 8) for j in range(NL)])
        return xn, base, link & zero_scr[...]

    def ln_full(c, xn_dst, base_dst):
        ln_stage(c)
        for r in range(NB):
            xn, base, _ = ln_block(r)
            xn_dst[r * RB:(r + 1) * RB, :] = xn
            base_dst[r * RB:(r + 1) * RB, :] = base

    def row_table(v):
        return jnp.concatenate([jnp.broadcast_to(v[j:j + 1, :], (8, 128)) for j in range(v.shape[0])], axis=1)

    def prep_params():
        dsk_scr[...] = row_table(par_v[0].astype(F32))
        lr = par_v[1].astype(F32)
        li = par_v[2].astype(F32)
        dt = _exp_expm1(par_v[3].astype(F32))[0].astype(BF16).astype(F32)
        a = dt * lr
        b = dt * li
        mag, magm1 = _exp_expm1(a)
        cb = jnp.cos(b)
        sh = jnp.sin(0.5 * b)
        lbr = mag * cb
        lbi = mag * jnp.sin(b)
        nr = magm1 * cb - 2.0 * (sh * sh)
        ni = lbi
        big = jnp.abs(lr) >= jnp.abs(li)
        r1 = li / lr
        d1 = lr + li * r1
        r2 = lr / li
        d2 = lr * r2 + li
        cr = jnp.where(big, (nr + ni * r1) / d1, (nr * r2 + ni) / d2)
        ci = jnp.where(big, (ni - nr * r1) / d1, (ni * r2 - nr) / d2)
        lam_scr[0] = row_table(lbr)
        lam_scr[1] = row_table(lbi)
        lam_scr[2] = row_table(2.0 * cr)
        lam_scr[3] = row_table(2.0 * ci)
        pr, pi = lbr, lbi
        n = 1
        while n < S:
            pr, pi = _cmul(pr, pi, pr, pi)
            n *= 2
        for k in range(3):
            pw_scr[2 * k] = row_table(pr)
            pw_scr[2 * k + 1] = row_table(pi)
            pr, pi = _cmul(pr, pi, pr, pi)
        carry_scr[...] = jnp.zeros(carry_scr.shape, F32)
        zero_scr[...] = jnp.zeros(zero_scr.shape, I32)

    def prep_c():
        cr = lam_scr[2, 0:1, :]
        ci = lam_scr[3, 0:1, :]
        RC = 64
        for r in range(0, D, RC):
            c_r = c_v[0, r:r + RC, :].astype(F32)
            c_i = c_v[1, r:r + RC, :].astype(F32)
            cp_scr[r:r + RC, :P] = (c_r * cr - c_i * ci).astype(BF16)
            cp_scr[r:r + RC, P:] = (-(c_r * ci) - c_i * cr).astype(BF16)

    def scan_tile(j, raw):
        sub = lax.broadcasted_iota(I32, (8, 128), 0)
        cr_ = slice(128 * j, 128 * (j + 1))
        ci_ = slice(P + 128 * j, P + 128 * (j + 1))
        lbr = lam_scr[0, :, cr_]
        lbi = lam_scr[1, :, cr_]
        er = raw[0:8, cr_]
        ei = raw[0:8, ci_]
        for t in range(1, S):
            ur = raw[8 * t:8 * t + 8, cr_]
            ui = raw[8 * t:8 * t + 8, ci_]
            er, ei = (lbr * er - lbi * ei) + ur, (lbr * ei + lbi * er) + ui
        vr = pltpu.roll(jnp.where(sub == 7, carry_scr[0, :, cr_], er), 1, 0)
        vi = pltpu.roll(jnp.where(sub == 7, carry_scr[1, :, cr_], ei), 1, 0)
        for k in range(3):
            sh = 1 << k
            tr, ti = _cmul(pw_scr[2 * k, :, cr_], pw_scr[2 * k + 1, :, cr_],
                           pltpu.roll(vr, sh, 0), pltpu.roll(vi, sh, 0))
            msk = sub >= sh
            vr = vr + jnp.where(msk, tr, 0.0)
            vi = vi + jnp.where(msk, ti, 0.0)
        hr, hi = vr, vi
        prs, pis = [], []
        for t2 in range(S // 2):
            outs = []
            for t in (2 * t2, 2 * t2 + 1):
                ur = raw[8 * t:8 * t + 8, cr_]
                ui = raw[8 * t:8 * t + 8, ci_]
                hr, hi = (lbr * hr - lbi * hi) + ur, (lbr * hi + lbi * hr) + ui
                outs.append((hr, hi))
            prs.append(jnp.concatenate([outs[0][0], outs[1][0]], axis=0).astype(BF16))
            pis.append(jnp.concatenate([outs[0][1], outs[1][1]], axis=0).astype(BF16))
        carry_scr[0, :, cr_] = hr
        carry_scr[1, :, cr_] = hi
        link = _or_all([pltpu.bitcast(v, I32) for pr_pi in zip(prs, pis) for v in pr_pi])
        return jnp.concatenate(prs, axis=0), jnp.concatenate(pis, axis=0), link & zero_scr[...]

    def up_stage(xn_ref, raw, wait):
        order = ORD_FIRST if wait else ORD_MAIN
        if wait:
            wait('wa')
        xn = xn_ref[...]
        hs, g_re, g_im = [], [], []
        for gi in range(NG):
            if wait and gi == NA:
                wait('wb')
                xn = xn_ref[...]
            lk = None
            if order[gi] == 'S':
                gr, gim, lk = scan_tile(len(g_re), raw)
                g_re.append(gr)
                g_im.append(gim)
            rs = slice(128 * gi, 128 * (gi + 1))
            if gi == 0 and not wait:
                gate = jnp.dot(xn, w1t_scr[...], preferred_element_type=F32)
            else:
                gate = lax.dot_general(xn, w1_v[rs, :], NT, preferred_element_type=F32)
            up = lax.dot_general(xn, w3_v[rs, :], NT, preferred_element_type=F32)
            hs.append(_pin(_swiglu(gate, up), lk))
        tail = lax.dot_general(xn, wt_v[...], NT, preferred_element_type=F32)
        ht = _swiglu(tail[:, :Ft], tail[:, Ft:])
        assert len(g_re) == NP
        return jnp.concatenate(hs, axis=1), ht, jnp.concatenate(g_re + g_im, axis=1)

    def write_out(out, c, tiles):
        for j in range(NL):
            for t in range(S):
                xout_scr[j, pl.ds(t, 8, stride=PITCH), :] = out[8 * t:8 * t + 8, 128 * j:128 * (j + 1)]
            for s in range(8):
                o_v[c & 1, S * s:S * (s + 1), 128 * j:128 * (j + 1)] = xout_scr[j, pl.ds(PITCH * s, S), :]
            if tiles:
                o_tile_copy(c, j).start()
        if not tiles:
            o_copy(c).start()

    def main(last):
        p = i & 1
        xn_p, base_p, raw_p = xn_scr.at[p], base_scr.at[p], raw_scr.at[p]
        if not last:
            ln_stage(i + 2)
        h, ht, g = up_stage(xn_p, raw_p, None)
        xns, bases = [], []

        def ln_pin(k):
            lk = None
            for _ in range(0 if last else LN_PINS[k]):
                r = len(xns)
                xb, bb, l2 = ln_block(r)
                xn_p[r * RB:(r + 1) * RB, :] = xb
                xns.append(xb)
                bases.append(bb)
                lk = l2 if lk is None else lk | l2
            return lk

        ys = []
        for n in range(NL):
            cs = slice(128 * n, 128 * (n + 1))
            yn = jnp.dot(h, w2_v[:Fm, cs], preferred_element_type=F32)
            yn = _pin32(yn, ln_pin(2 * n))
            yn = yn + jnp.dot(ht, w2_v[Fm:, cs], preferred_element_type=F32)
            yn = yn + lax.dot_general(g, cp_scr[cs, :], NT, preferred_element_type=F32)
            yn = _pin32(yn, ln_pin(2 * n + 1))
            ys.append(yn)
        y = jnp.concatenate(ys, axis=1)
        if not last:
            assert len(xns) == NB
            xn_next = jnp.concatenate(xns, axis=0)
            raw_p[:, :P] = lax.dot_general(xn_next, b_v[0], NT, preferred_element_type=F32)
            raw_p[:, P:] = lax.dot_general(xn_next, b_v[1], NT, preferred_element_type=F32)
        out = base_p[...] + y
        if not last:
            base_p[...] = jnp.concatenate(bases, axis=0)
        write_out(out, i, last)

    def first_step():
        cps = weight_copies()

        def wait(name):
            for cp in cps[name]:
                cp.wait()

        for cp in cps['par']:
            cp.start()
        x_copy(0).start()
        for name in cps:
            if name != 'par':
                for cp in cps[name]:
                    cp.start()
        x_copy(3).start()
        wait('par')
        prep_params()
        x_copy(0).wait()
        ln_full(0, xn0_scr, base0_scr)
        xn1, base1, raw1 = xn_scr.at[1], base_scr.at[1], raw_scr.at[1]
        xn2, base2, raw2 = xn_scr.at[0], base_scr.at[0], raw_scr.at[0]

        PA = N0 * 128
        PB, PL = PA - 128, P - 128

        def bdot(xr, k0, k1, w, n0, n1):
            return lax.dot_general(xr[:, k0:k1], b_v[w, n0:n1, k0:k1], NT, preferred_element_type=F32)

        def ln_feeder(xn_dst, base_dst):
            xns = []

            def nxt(cnt=1):
                lk = None
                for _ in range(cnt):
                    if len(xns) < NB:
                        r = len(xns)
                        xb, bb, l2 = ln_block(r)
                        xn_dst[r * RB:(r + 1) * RB, :] = xb
                        base_dst[r * RB:(r + 1) * RB, :] = bb
                        xns.append(xb)
                        lk = l2 if lk is None else lk | l2
                return lk
            return xns, nxt

        wait('b0')
        raw0_scr[:, :PB] = bdot(xn0_scr, 0, D, 0, 0, PB)
        raw0_scr[:, PB:PA] = bdot(xn0_scr, 0, K0 * 128, 0, PB, PA)
        wait('b1')
        ln_stage(1)
        xns, nxt = ln_feeder(xn1, base1)
        raw0_scr[:, PB:PA] += bdot(xn0_scr, K0 * 128, D, 0, PB, PA)
        raw0_scr[:, PA:P] = bdot(xn0_scr, 0, D, 0, PA, P)
        nxt(NB)
        xx = jnp.concatenate(xns, axis=0)
        raw1[:, :PL] = bdot(xx, 0, D, 0, 0, PL)
        raw1[:, PL:P] = bdot(xx, 0, K1 * 128, 0, PL, P)
        wait('b2')
        ln_stage(2)
        xns, nxt = ln_feeder(xn2, base2)
        jobs = [(xn0_scr, raw0_scr, n) for n in range(NP)] + [(xn1, raw1, n) for n in range(NP - 1)]
        for q, (xr, rw, n) in enumerate(jobs):
            lk = nxt() if q >= 1 else None
            res = bdot(xr, 0, D, 1, 128 * n, 128 * (n + 1))
            rw[:, P + 128 * n:P + 128 * (n + 1)] = _pin32(res, lk)
        raw1[:, PL:P] += bdot(xn1, K1 * 128, D, 0, PL, P)
        raw1[:, P + PL:] = bdot(xn1, 0, K2 * 128, 1, PL, P)
        assert len(xns) == NB
        xx = jnp.concatenate(xns, axis=0)
        raw2[:, :P] = lax.dot_general(xx, b_v[0], NT, preferred_element_type=F32)
        raw2[:, P:] = lax.dot_general(xx, b_v[1], NT, preferred_element_type=F32)

        h, ht, g = up_stage(xn0_scr, raw0_scr, wait)
        raw1[:, P + PL:] += bdot(xn1, K2 * 128, D, 1, PL, P)
        w1t_scr[...] = w1_v[0:128, :].astype(F32).T.astype(BF16)
        ys = []
        for n in range(NL):
            if n == ND:
                wait('c')
                prep_c()
            cs = slice(128 * n, 128 * (n + 1))
            yn = jnp.dot(h, w2_v[:Fm, cs], preferred_element_type=F32)
            yn = yn + jnp.dot(ht, w2_v[Fm:, cs], preferred_element_type=F32)
            ys.append(yn)
        y = jnp.concatenate(ys, axis=1)
        y = y + lax.dot_general(g, cp_scr[...], NT, preferred_element_type=F32)
        write_out(base0_scr[...] + y, 0, False)

    @pl.when(i == 0)
    def _():
        first_step()
        x_copy(3).wait()

    @pl.when(jnp.logical_and(i > 0, i < NC - 2))
    def _():
        more_x = i + 3 < NC
        x_next = x_copy(jnp.minimum(i + 3, NC - 1))
        o_prev = o_copy(i - 1)

        @pl.when(more_x)
        def _():
            x_next.start()
        main(False)

        @pl.when(more_x)
        def _():
            x_next.wait()
        o_prev.wait()

    @pl.when(i >= NC - 2)
    def _():
        o_prev = o_copy(i - 1)
        main(True)
        o_prev.wait()

        @pl.when(i == NC - 1)
        def _():
            o_copy(NC - 1).wait()


@jax.jit
def pallas_parallel_sum__ssm_conv_s5__glu_gated_swiglu__prompt_kernel(
    A_x: jax.Array,
    A_Lambda_re: jax.Array,
    A_Lambda_im: jax.Array,
    A_B_re: jax.Array,
    A_B_im: jax.Array,
    A_C_re: jax.Array,
    A_C_im: jax.Array,
    A_log_dt: jax.Array,
    A_Dskip: jax.Array,
    B_x: jax.Array,
    B_w1: jax.Array,
    B_w3: jax.Array,
    B_w2: jax.Array,
):
    del B_x
    Bsz, L, D = A_x.shape
    P = A_Lambda_re.shape[0]
    Fh = B_w1.shape[1]
    Ft = Fh % 128
    Fm = Fh - Ft
    NC = L // T
    assert Bsz == 1 and L % T == 0 and NC >= 4 and D % 128 == 0 and P == D and Ft == 64
    assert Fm // 128 == len(ORD_MAIN) and P // 128 == ORD_MAIN.count('S') and 2 * (D // 128) == len(LN_PINS)
    vec = lambda a: a.reshape(-1, 128)
    args = (A_x, vec(A_Lambda_re), vec(A_Lambda_im), vec(A_log_dt), vec(A_Dskip),
            A_B_re, A_B_im, A_C_re, A_C_im, B_w1.T, B_w3.T, B_w2)
    return pl.pallas_call(
        _kernel,
        grid=(NC,),
        in_specs=[pl.BlockSpec(memory_space=pl.ANY)] * len(args),
        out_specs=pl.BlockSpec(memory_space=pl.ANY),
        out_shape=jax.ShapeDtypeStruct((Bsz, L, D), F32),
        scratch_shapes=[
            pltpu.VMEM((L, D), BF16),
            pltpu.VMEM((4, P // 128, 128), BF16),
            pltpu.VMEM((2, P, D), BF16),
            pltpu.VMEM((2, D, P), BF16),
            pltpu.VMEM((Fm, D), BF16),
            pltpu.VMEM((Fm, D), BF16),
            pltpu.VMEM((2 * Ft, D), BF16),
            pltpu.VMEM((Fh, D), BF16),
            pltpu.VMEM((D // 128, 8 * PITCH, 128), F32),
            pltpu.VMEM((D // 128, 8 * PITCH, 128), F32),
            pltpu.VMEM((2, T, D), F32),
            pltpu.VMEM((2, T, D), BF16),
            pltpu.VMEM((2, T, D), F32),
            pltpu.VMEM((2, T, 2 * P), F32),
            pltpu.VMEM((T, D), BF16),
            pltpu.VMEM((T, D), F32),
            pltpu.VMEM((T, 2 * P), F32),
            pltpu.VMEM((8, D), F32),
            pltpu.VMEM((4, 8, P), F32),
            pltpu.VMEM((6, 8, P), F32),
            pltpu.VMEM((D, 2 * P), BF16),
            pltpu.VMEM((2, 8, P), F32),
            pltpu.VMEM((8, 128), I32),
            pltpu.VMEM((D, 128), BF16),
            pltpu.SemaphoreType.DMA((N_SEM,)),
        ],
        compiler_params=pltpu.CompilerParams(dimension_semantics=("arbitrary",),
                                             vmem_limit_bytes=64 * 1024 * 1024),
    )(*args)
```

```python
import jax
import jax.numpy as jnp
from jax import lax
import jax.experimental.pallas as pl
import jax.experimental.pallas.tpu as pltpu

F32 = jnp.float32
BF16 = jnp.bfloat16
I32 = jnp.int32
NT = (((1,), (1,)), ((), ()))

T = 256
S = T // 8
PITCH = S + 4
RB = 32
NB = T // RB
N0, K0, K1, K2, NA, ND = 3, 3, 4, 4, 10, 2
ORD_FIRST = '-S-S-S-S-S---'
ORD_MAIN = 'S-S-S-S-S----'
LN_PINS = (1, 1, 1, 1, 1, 1, 1, 1, 0, 0)
S_PAR, S_X, S_B0, S_B1, S_B2, S_WA, S_WB, S_C, S_O, N_SEM = 0, 1, 3, 4, 5, 6, 7, 8, 9, 11


def _cmul(ar, ai, br, bi):
    return ar * br - ai * bi, ar * bi + ai * br


def _exp_expm1(a):
    ac = jnp.clip(a, -104.0, 89.0)
    k = jnp.floor(ac * 1.4426950408889634 + 0.5)
    r = (ac - k * 0.693145751953125) - k * 1.42860682030941723212e-6
    p = 1.0 / 40320.0
    for c in (1.0 / 5040.0, 1.0 / 720.0, 1.0 / 120.0, 1.0 / 24.0, 1.0 / 6.0, 0.5):
        p = p * r + c
    p = (p * r) * r + r
    ki = k.astype(I32)
    k1 = ki >> 1
    s1 = pltpu.bitcast((k1 + 127) << 23, F32)
    s2 = pltpu.bitcast((ki - k1 + 127) << 23, F32)
    e = (s1 * (1.0 + p)) * s2
    return e, jnp.where(ki == 0, p, e - 1.0)


def _swiglu(g, u):
    hg = 0.5 * g
    return ((hg * jnp.tanh(hg) + hg) * u).astype(BF16)


def _or_all(vs):
    acc = vs[0]
    for v in vs[1:]:
        acc = acc | v
    return acc


def _pin(v, link):
    if link is None:
        return v
    blk = pltpu.bitcast(pltpu.bitcast(v[0:16, :], I32) | link, BF16)
    return jnp.concatenate([blk, v[16:, :]], axis=0)


def _pin32(v, link):
    if link is None:
        return v
    blk = pltpu.bitcast(pltpu.bitcast(v[0:8, :], I32) | link, F32)
    return jnp.concatenate([blk, v[8:, :]], axis=0)


def _kernel(x_hbm, lre_hbm, lim_hbm, ldt_hbm, dsk_hbm, bre_hbm, bim_hbm, cre_hbm, cim_hbm,
            w1_hbm, w3_hbm, w2_hbm, o_hbm,
            x_v, par_v, b_v, c_v, w1_v, w3_v, wt_v, w2_v,
            xin_scr, xout_scr, o_v, xn_scr, base_scr, raw_scr, xn0_scr, base0_scr, raw0_scr,
            dsk_scr, lam_scr, pw_scr, cp_scr, carry_scr, zero_scr, w1t_scr, sem):
    L, D = x_v.shape
    P = b_v.shape[1]
    Fh = w2_v.shape[0]
    Fm = (Fh // 128) * 128
    Ft = Fh - Fm
    NG, NL, NP, NC = Fm // 128, D // 128, P // 128, L // T
    i = pl.program_id(0)

    def x_copy(c, slot=None):
        slot = S_X + (c & 1) if slot is None else slot
        return pltpu.make_async_copy(x_hbm.at[0, pl.ds(c * T, T), :], x_v.at[pl.ds(c * T, T), :], sem.at[slot])

    def o_copy(c):
        return pltpu.make_async_copy(o_v.at[c & 1], o_hbm.at[0, pl.ds(c * T, T), :], sem.at[S_O + (c & 1)])

    def o_tile_copy(c, j):
        cs = pl.ds(128 * j, 128)
        return pltpu.make_async_copy(o_v.at[c & 1, :, cs], o_hbm.at[0, pl.ds(c * T, T), cs],
                                     sem.at[S_O + (c & 1)])

    def weight_copies():
        cps = {}

        def add(name, slot, src, dst):
            cps.setdefault(name, []).append(pltpu.make_async_copy(src, dst, sem.at[slot]))

        for k, r in enumerate((dsk_hbm, lre_hbm, lim_hbm, ldt_hbm)):
            add('par', S_PAR, r, par_v.at[k])
        PA, FA, WD = N0 * 128, NA * 128, ND * 128
        add('b0', S_B0, bre_hbm.at[pl.ds(0, PA), :], b_v.at[0, pl.ds(0, PA), :])
        cps['b1'] = [x_copy(1, S_B1)]
        add('b1', S_B1, bre_hbm.at[pl.ds(PA, P - PA), :], b_v.at[0, pl.ds(PA, P - PA), :])
        cps['b2'] = [x_copy(2, S_B2)]
        add('b2', S_B2, bim_hbm, b_v.at[1])
        add('wa', S_WA, w1_hbm.at[pl.ds(0, FA), :], w1_v.at[pl.ds(0, FA), :])
        add('wa', S_WA, w3_hbm.at[pl.ds(0, FA), :], w3_v.at[pl.ds(0, FA), :])
        add('wb', S_WB, w1_hbm.at[pl.ds(FA, Fm - FA), :], w1_v.at[pl.ds(FA, Fm - FA), :])
        add('wb', S_WB, w3_hbm.at[pl.ds(FA, Fm - FA), :], w3_v.at[pl.ds(FA, Fm - FA), :])
        add('wb', S_WB, w1_hbm.at[pl.ds(Fm, Ft), :], wt_v.at[pl.ds(0, Ft), :])
        add('wb', S_WB, w3_hbm.at[pl.ds(Fm, Ft), :], wt_v.at[pl.ds(Ft, Ft), :])
        add('wb', S_WB, w2_hbm.at[:, pl.ds(0, WD)], w2_v.at[:, pl.ds(0, WD)])
        add('c', S_C, w2_hbm.at[:, pl.ds(WD, D - WD)], w2_v.at[:, pl.ds(WD, D - WD)])
        add('c', S_C, cre_hbm, c_v.at[0])
        add('c', S_C, cim_hbm, c_v.at[1])
        return cps

    def ln_stage(c):
        start = c * T if isinstance(c, int) else pl.multiple_of(c * T, T)
        xf = x_v[pl.ds(start, T), :].astype(F32)
        for j in range(NL):
            for s in range(8):
                xin_scr[j, pl.ds(PITCH * s, S), :] = xf[S * s:S * (s + 1), 128 * j:128 * (j + 1)]

    def ln_block(r):
        ts = range(r * RB // 8, (r + 1) * RB // 8)
        xp = jnp.concatenate(
            [jnp.concatenate([xin_scr[j, pl.ds(t, 8, stride=PITCH), :] for t in ts], axis=0)
             for j in range(NL)], axis=1)
        mean = jnp.sum(xp, axis=-1, keepdims=True) * (1.0 / D)
        xc = xp - mean
        var = jnp.sum(xc * xc, axis=-1, keepdims=True) * (1.0 / D)
        m_b = mean.astype(BF16).astype(F32)
        v_b = var.astype(BF16).astype(F32)
        sd = jnp.sqrt((v_b + 1e-5).astype(BF16).astype(F32)).astype(BF16).astype(F32)
        xn = ((xp - m_b) * (1.0 / sd)).astype(BF16)
        base = xp + xn.astype(F32) * dsk_scr[0:1, :]
        bi = pltpu.bitcast(base, I32)
        link = _or_all([bi[8 * a:8 * a + 8, 128 * j:128 * (j + 1)] for a in range(RB // 8) for j in range(NL)])
        return xn, base, link & zero_scr[...]

    def ln_full(c, xn_dst, base_dst):
        ln_stage(c)
        for r in range(NB):
            xn, base, _ = ln_block(r)
            xn_dst[r * RB:(r + 1) * RB, :] = xn
            base_dst[r * RB:(r + 1) * RB, :] = base

    def row_table(v):
        return jnp.concatenate([jnp.broadcast_to(v[j:j + 1, :], (8, 128)) for j in range(v.shape[0])], axis=1)

    def prep_params():
        dsk_scr[...] = row_table(par_v[0].astype(F32))
        lr = par_v[1].astype(F32)
        li = par_v[2].astype(F32)
        dt = _exp_expm1(par_v[3].astype(F32))[0].astype(BF16).astype(F32)
        a = dt * lr
        b = dt * li
        mag, magm1 = _exp_expm1(a)
        cb = jnp.cos(b)
        sh = jnp.sin(0.5 * b)
        lbr = mag * cb
        lbi = mag * jnp.sin(b)
        nr = magm1 * cb - 2.0 * (sh * sh)
        ni = lbi
        big = jnp.abs(lr) >= jnp.abs(li)
        r1 = li / lr
        d1 = lr + li * r1
        r2 = lr / li
        d2 = lr * r2 + li
        cr = jnp.where(big, (nr + ni * r1) / d1, (nr * r2 + ni) / d2)
        ci = jnp.where(big, (ni - nr * r1) / d1, (ni * r2 - nr) / d2)
        lam_scr[0] = row_table(lbr)
        lam_scr[1] = row_table(lbi)
        lam_scr[2] = row_table(2.0 * cr)
        lam_scr[3] = row_table(2.0 * ci)
        pr, pi = lbr, lbi
        n = 1
        while n < S:
            pr, pi = _cmul(pr, pi, pr, pi)
            n *= 2
        for k in range(3):
            pw_scr[2 * k] = row_table(pr)
            pw_scr[2 * k + 1] = row_table(pi)
            pr, pi = _cmul(pr, pi, pr, pi)
        carry_scr[...] = jnp.zeros(carry_scr.shape, F32)
        zero_scr[...] = jnp.zeros(zero_scr.shape, I32)

    def prep_c():
        cr = lam_scr[2, 0:1, :]
        ci = lam_scr[3, 0:1, :]
        RC = 64
        for r in range(0, D, RC):
            c_r = c_v[0, r:r + RC, :].astype(F32)
            c_i = c_v[1, r:r + RC, :].astype(F32)
            cp_scr[r:r + RC, :P] = (c_r * cr - c_i * ci).astype(BF16)
            cp_scr[r:r + RC, P:] = (-(c_r * ci) - c_i * cr).astype(BF16)

    def scan_tile(j, raw):
        sub = lax.broadcasted_iota(I32, (8, 128), 0)
        cr_ = slice(128 * j, 128 * (j + 1))
        ci_ = slice(P + 128 * j, P + 128 * (j + 1))
        lbr = lam_scr[0, :, cr_]
        lbi = lam_scr[1, :, cr_]
        er = raw[0:8, cr_]
        ei = raw[0:8, ci_]
        for t in range(1, S):
            ur = raw[8 * t:8 * t + 8, cr_]
            ui = raw[8 * t:8 * t + 8, ci_]
            er, ei = (lbr * er - lbi * ei) + ur, (lbr * ei + lbi * er) + ui
        vr = pltpu.roll(jnp.where(sub == 7, carry_scr[0, :, cr_], er), 1, 0)
        vi = pltpu.roll(jnp.where(sub == 7, carry_scr[1, :, cr_], ei), 1, 0)
        for k in range(3):
            sh = 1 << k
            tr, ti = _cmul(pw_scr[2 * k, :, cr_], pw_scr[2 * k + 1, :, cr_],
                           pltpu.roll(vr, sh, 0), pltpu.roll(vi, sh, 0))
            msk = sub >= sh
            vr = vr + jnp.where(msk, tr, 0.0)
            vi = vi + jnp.where(msk, ti, 0.0)
        hr, hi = vr, vi
        prs, pis = [], []
        for t2 in range(S // 2):
            outs = []
            for t in (2 * t2, 2 * t2 + 1):
                ur = raw[8 * t:8 * t + 8, cr_]
                ui = raw[8 * t:8 * t + 8, ci_]
                hr, hi = (lbr * hr - lbi * hi) + ur, (lbr * hi + lbi * hr) + ui
                outs.append((hr, hi))
            prs.append(jnp.concatenate([outs[0][0], outs[1][0]], axis=0).astype(BF16))
            pis.append(jnp.concatenate([outs[0][1], outs[1][1]], axis=0).astype(BF16))
        carry_scr[0, :, cr_] = hr
        carry_scr[1, :, cr_] = hi
        link = _or_all([pltpu.bitcast(v, I32) for pr_pi in zip(prs, pis) for v in pr_pi])
        return jnp.concatenate(prs, axis=0), jnp.concatenate(pis, axis=0), link & zero_scr[...]

    def up_stage(xn_ref, raw, wait):
        order = ORD_FIRST if wait else ORD_MAIN
        if wait:
            wait('wa')
        xn = xn_ref[...]
        hs, g_re, g_im = [], [], []
        for gi in range(NG):
            if wait and gi == NA:
                wait('wb')
                xn = xn_ref[...]
            lk = None
            if order[gi] == 'S':
                gr, gim, lk = scan_tile(len(g_re), raw)
                g_re.append(gr)
                g_im.append(gim)
            rs = slice(128 * gi, 128 * (gi + 1))
            if gi == 0 and not wait:
                gate = jnp.dot(xn, w1t_scr[...], preferred_element_type=F32)
            else:
                gate = lax.dot_general(xn, w1_v[rs, :], NT, preferred_element_type=F32)
            up = lax.dot_general(xn, w3_v[rs, :], NT, preferred_element_type=F32)
            hs.append(_pin(_swiglu(gate, up), lk))
        tail = lax.dot_general(xn, wt_v[...], NT, preferred_element_type=F32)
        ht = _swiglu(tail[:, :Ft], tail[:, Ft:])
        assert len(g_re) == NP
        return jnp.concatenate(hs, axis=1), ht, jnp.concatenate(g_re + g_im, axis=1)

    def write_out(out, c, tiles):
        for j in range(NL):
            for t in range(S):
                xout_scr[j, pl.ds(t, 8, stride=PITCH), :] = out[8 * t:8 * t + 8, 128 * j:128 * (j + 1)]
            for s in range(8):
                o_v[c & 1, S * s:S * (s + 1), 128 * j:128 * (j + 1)] = xout_scr[j, pl.ds(PITCH * s, S), :]
            if tiles:
                o_tile_copy(c, j).start()
        if not tiles:
            o_copy(c).start()

    def main(last):
        p = i & 1
        xn_p, base_p, raw_p = xn_scr.at[p], base_scr.at[p], raw_scr.at[p]
        if not last:
            ln_stage(i + 2)
        h, ht, g = up_stage(xn_p, raw_p, None)
        xns, bases = [], []

        def ln_pin(k):
            lk = None
            for _ in range(0 if last else LN_PINS[k]):
                r = len(xns)
                xb, bb, l2 = ln_block(r)
                xn_p[r * RB:(r + 1) * RB, :] = xb
                xns.append(xb)
                bases.append(bb)
                lk = l2 if lk is None else lk | l2
            return lk

        ys = []
        for n in range(NL):
            cs = slice(128 * n, 128 * (n + 1))
            yn = jnp.dot(h, w2_v[:Fm, cs], preferred_element_type=F32)
            yn = _pin32(yn, ln_pin(2 * n))
            yn = yn + jnp.dot(ht, w2_v[Fm:, cs], preferred_element_type=F32)
            yn = yn + lax.dot_general(g, cp_scr[cs, :], NT, preferred_element_type=F32)
            yn = _pin32(yn, ln_pin(2 * n + 1))
            ys.append(yn)
        y = jnp.concatenate(ys, axis=1)
        if not last:
            assert len(xns) == NB
            xn_next = jnp.concatenate(xns, axis=0)
            raw_p[:, :P] = lax.dot_general(xn_next, b_v[0], NT, preferred_element_type=F32)
            raw_p[:, P:] = lax.dot_general(xn_next, b_v[1], NT, preferred_element_type=F32)
        out = base_p[...] + y
        if not last:
            base_p[...] = jnp.concatenate(bases, axis=0)
        write_out(out, i, last)

    def first_step():
        cps = weight_copies()

        def wait(name):
            for cp in cps[name]:
                cp.wait()

        for cp in cps['par']:
            cp.start()
        x_copy(0).start()
        for name in cps:
            if name != 'par':
                for cp in cps[name]:
                    cp.start()
        x_copy(3).start()
        wait('par')
        prep_params()
        x_copy(0).wait()
        ln_full(0, xn0_scr, base0_scr)
        xn1, base1, raw1 = xn_scr.at[1], base_scr.at[1], raw_scr.at[1]
        xn2, base2, raw2 = xn_scr.at[0], base_scr.at[0], raw_scr.at[0]

        PA = N0 * 128
        PB, PL = PA - 128, P - 128

        def bdot(xr, k0, k1, w, n0, n1):
            return lax.dot_general(xr[:, k0:k1], b_v[w, n0:n1, k0:k1], NT, preferred_element_type=F32)

        def ln_feeder(xn_dst, base_dst):
            xns = []

            def nxt(cnt=1):
                lk = None
                for _ in range(cnt):
                    if len(xns) < NB:
                        r = len(xns)
                        xb, bb, l2 = ln_block(r)
                        xn_dst[r * RB:(r + 1) * RB, :] = xb
                        base_dst[r * RB:(r + 1) * RB, :] = bb
                        xns.append(xb)
                        lk = l2 if lk is None else lk | l2
                return lk
            return xns, nxt

        wait('b0')
        raw0_scr[:, :PB] = bdot(xn0_scr, 0, D, 0, 0, PB)
        raw0_scr[:, PB:PA] = bdot(xn0_scr, 0, K0 * 128, 0, PB, PA)
        wait('b1')
        ln_stage(1)
        xns, nxt = ln_feeder(xn1, base1)
        raw0_scr[:, PB:PA] += bdot(xn0_scr, K0 * 128, D, 0, PB, PA)
        raw0_scr[:, PA:P] = bdot(xn0_scr, 0, D, 0, PA, P)
        nxt(NB)
        xx = jnp.concatenate(xns, axis=0)
        raw1[:, :PL] = bdot(xx, 0, D, 0, 0, PL)
        raw1[:, PL:P] = bdot(xx, 0, K1 * 128, 0, PL, P)
        wait('b2')
        ln_stage(2)
        xns, nxt = ln_feeder(xn2, base2)
        jobs = [(xn0_scr, raw0_scr, n) for n in range(NP)] + [(xn1, raw1, n) for n in range(NP - 1)]
        for q, (xr, rw, n) in enumerate(jobs):
            lk = nxt() if q >= 1 else None
            res = bdot(xr, 0, D, 1, 128 * n, 128 * (n + 1))
            rw[:, P + 128 * n:P + 128 * (n + 1)] = _pin32(res, lk)
        raw1[:, PL:P] += bdot(xn1, K1 * 128, D, 0, PL, P)
        raw1[:, P + PL:] = bdot(xn1, 0, K2 * 128, 1, PL, P)
        assert len(xns) == NB
        xx = jnp.concatenate(xns, axis=0)
        raw2[:, :P] = lax.dot_general(xx, b_v[0], NT, preferred_element_type=F32)
        raw2[:, P:] = lax.dot_general(xx, b_v[1], NT, preferred_element_type=F32)

        h, ht, g = up_stage(xn0_scr, raw0_scr, wait)
        raw1[:, P + PL:] += bdot(xn1, K2 * 128, D, 1, PL, P)
        w1t_scr[...] = w1_v[0:128, :].astype(F32).T.astype(BF16)
        ys = []
        for n in range(NL):
            if n == ND:
                wait('c')
                prep_c()
            cs = slice(128 * n, 128 * (n + 1))
            yn = jnp.dot(h, w2_v[:Fm, cs], preferred_element_type=F32)
            yn = yn + jnp.dot(ht, w2_v[Fm:, cs], preferred_element_type=F32)
            ys.append(yn)
        y = jnp.concatenate(ys, axis=1)
        y = y + lax.dot_general(g, cp_scr[...], NT, preferred_element_type=F32)
        write_out(base0_scr[...] + y, 0, False)

    @pl.when(i == 0)
    def _():
        first_step()
        x_copy(3).wait()

    @pl.when(jnp.logical_and(i > 0, i < NC - 2))
    def _():
        more_x = i + 3 < NC
        x_next = x_copy(jnp.minimum(i + 3, NC - 1))
        o_prev = o_copy(i - 1)

        @pl.when(more_x)
        def _():
            x_next.start()
        main(False)

        @pl.when(more_x)
        def _():
            x_next.wait()
        o_prev.wait()

    @pl.when(i >= NC - 2)
    def _():
        o_prev = o_copy(i - 1)
        main(True)
        o_prev.wait()

        @pl.when(i == NC - 1)
        def _():
            o_copy(NC - 1).wait()


def _compiler_params():
    kw = dict(dimension_semantics=("arbitrary",), vmem_limit_bytes=64 * 1024 * 1024)
    try:
        return pltpu.CompilerParams(disable_bounds_checks=True, disable_semaphore_checks=True, **kw)
    except TypeError:
        return pltpu.CompilerParams(**kw)


@jax.jit
def pallas_parallel_sum__ssm_conv_s5__glu_gated_swiglu__prompt_kernel(
    A_x: jax.Array,
    A_Lambda_re: jax.Array,
    A_Lambda_im: jax.Array,
    A_B_re: jax.Array,
    A_B_im: jax.Array,
    A_C_re: jax.Array,
    A_C_im: jax.Array,
    A_log_dt: jax.Array,
    A_Dskip: jax.Array,
    B_x: jax.Array,
    B_w1: jax.Array,
    B_w3: jax.Array,
    B_w2: jax.Array,
):
    del B_x
    Bsz, L, D = A_x.shape
    P = A_Lambda_re.shape[0]
    Fh = B_w1.shape[1]
    Ft = Fh % 128
    Fm = Fh - Ft
    NC = L // T
    assert Bsz == 1 and L % T == 0 and NC >= 4 and D % 128 == 0 and P == D and Ft == 64
    assert Fm // 128 == len(ORD_MAIN) and P // 128 == ORD_MAIN.count('S') and 2 * (D // 128) == len(LN_PINS)
    vec = lambda a: a.reshape(-1, 128)
    args = (A_x, vec(A_Lambda_re), vec(A_Lambda_im), vec(A_log_dt), vec(A_Dskip),
            A_B_re, A_B_im, A_C_re, A_C_im, B_w1.T, B_w3.T, B_w2)
    return pl.pallas_call(
        _kernel,
        grid=(NC,),
        in_specs=[pl.BlockSpec(memory_space=pl.ANY)] * len(args),
        out_specs=pl.BlockSpec(memory_space=pl.ANY),
        out_shape=jax.ShapeDtypeStruct((Bsz, L, D), F32),
        scratch_shapes=[
            pltpu.VMEM((L, D), BF16),
            pltpu.VMEM((4, P // 128, 128), BF16),
            pltpu.VMEM((2, P, D), BF16),
            pltpu.VMEM((2, D, P), BF16),
            pltpu.VMEM((Fm, D), BF16),
            pltpu.VMEM((Fm, D), BF16),
            pltpu.VMEM((2 * Ft, D), BF16),
            pltpu.VMEM((Fh, D), BF16),
            pltpu.VMEM((D // 128, 8 * PITCH, 128), F32),
            pltpu.VMEM((D // 128, 8 * PITCH, 128), F32),
            pltpu.VMEM((2, T, D), F32),
            pltpu.VMEM((2, T, D), BF16),
            pltpu.VMEM((2, T, D), F32),
            pltpu.VMEM((2, T, 2 * P), F32),
            pltpu.VMEM((T, D), BF16),
            pltpu.VMEM((T, D), F32),
            pltpu.VMEM((T, 2 * P), F32),
            pltpu.VMEM((8, D), F32),
            pltpu.VMEM((4, 8, P), F32),
            pltpu.VMEM((6, 8, P), F32),
            pltpu.VMEM((D, 2 * P), BF16),
            pltpu.VMEM((2, 8, P), F32),
            pltpu.VMEM((8, 128), I32),
            pltpu.VMEM((D, 128), BF16),
            pltpu.SemaphoreType.DMA((N_SEM,)),
        ],
        compiler_params=_compiler_params(),
    )(*args)
```
